```python
import jax
import jax.numpy as jnp

def _softmax(x, axis=-1):
    return jax.nn.softmax(x, axis=axis)

def _gelu(x):
    return jax.nn.gelu(x, approximate=True)

def _silu(x):
    return jax.nn.silu(x)

def _sigmoid(x):
    return jax.nn.sigmoid(x)

def _layernorm(x, axis=-1, eps=1e-05):
    m = jnp.mean(x, axis=axis, keepdims=True)
    v = jnp.var(x, axis=axis, keepdims=True)
    return (x - m) / jnp.sqrt(v + eps)

def _scatter_add(tgt, idx, src, axis=0):
    return tgt.at[idx].add(src)

def _segment_sum(src, seg, n):
    return jax.ops.segment_sum(src, seg, n)

class _Rng:

    def __init__(self, key):
        self._k = key

    def _next(self):
        self._k, sub = jax.random.split(self._k)
        return sub

    def normal(self, shape):
        return jax.random.normal(self._next(), shape, dtype=jnp.bfloat16)

    def randint(self, lo, hi, shape):
        return jax.random.randint(self._next(), shape, lo, hi, dtype=jnp.int32)

    def uniform(self, shape, lo=0.0, hi=1.0):
        return jax.random.uniform(self._next(), shape, jnp.bfloat16, lo, hi)

    def permutation(self, n):
        return jax.random.permutation(self._next(), n)
kernel_name = 'standalone__conformer_family_conformer__speech'

def setup_inputs():
    _rng = _Rng(jax.random.key(int.from_bytes(__import__("os").urandom(4), "little")))
    _w = lambda a: (lambda t: t.astype(jnp.bfloat16) if jnp.issubdtype(t.dtype, jnp.floating) else t)(jnp.asarray(a))
    B, T, D, K = (2, 4000, 512, 15)
    F = 4 * D
    s = D ** (-0.5)
    sf = F ** (-0.5)
    return {'x': _w((lambda *s: _rng.normal(s) * 0.05)(B, T, D)), 'w_ff1_a': _w((lambda *s: _rng.normal(s) * 0.05)(D, F) * s), 'w_ff1_b': _w((lambda *s: _rng.normal(s) * 0.05)(F, D) * sf), 'w_q': _w((lambda *s: _rng.normal(s) * 0.05)(D, D) * s), 'w_k': _w((lambda *s: _rng.normal(s) * 0.05)(D, D) * s), 'w_v': _w((lambda *s: _rng.normal(s) * 0.05)(D, D) * s), 'w_o': _w((lambda *s: _rng.normal(s) * 0.05)(D, D) * s), 'w_pw1': _w((lambda *s: _rng.normal(s) * 0.05)(D, 2 * D) * s), 'dw': _w((lambda *s: _rng.normal(s) * 0.05)(K, D) * K ** (-0.5)), 'w_pw2': _w((lambda *s: _rng.normal(s) * 0.05)(D, D) * s), 'w_ff2_a': _w((lambda *s: _rng.normal(s) * 0.05)(D, F) * s), 'w_ff2_b': _w((lambda *s: _rng.normal(s) * 0.05)(F, D) * sf)}

def reference(x, w_ff1_a, w_ff1_b, w_q, w_k, w_v, w_o, w_pw1, dw, w_pw2, w_ff2_a, w_ff2_b):
    B, T, D = x.shape
    K = dw.shape[0]
    scale = D ** (-0.5)
    h = _layernorm(x, axis=-1)
    h = _silu(h @ w_ff1_a) @ w_ff1_b
    x1 = x + 0.5 * h
    h = _layernorm(x1, axis=-1)
    q = h @ w_q
    k = h @ w_k
    v = h @ w_v
    scores = jnp.einsum('btd,bsd->bts', q, k) * scale
    p = _softmax(scores, axis=-1)
    attn = jnp.einsum('bts,bsd->btd', p, v) @ w_o
    x2 = x1 + attn
    h = _layernorm(x2, axis=-1)
    h = h @ w_pw1
    a = h[..., :D].copy()
    b = h[..., D:].copy()
    h = a * _sigmoid(b)
    pad = K // 2
    hp = jnp.pad(h, ((0, 0), (pad, K - 1 - pad), (0, 0)))
    dc = jnp.zeros_like(h)
    for i in range(K):
        dc = dc + hp[:, i:i + T, :] * dw[i][None, None, :]
    flat = dc.reshape(-1, D)
    mu = flat.mean(0)
    var = ((flat - mu) ** 2).mean(0)
    dc = (dc - mu[None, None, :]) / jnp.sqrt(var[None, None, :] + 1e-05)
    h = _silu(dc) @ w_pw2
    x3 = x2 + h
    h = _layernorm(x3, axis=-1)
    h = _silu(h @ w_ff2_a) @ w_ff2_b
    x4 = x3 + 0.5 * h
    return _layernorm(x4, axis=-1)
```

```python
import math
import numpy as np
import jax
import jax.numpy as jnp
from jax import lax
import jax.experimental.pallas as pl
import jax.experimental.pallas.tpu as pltpu

CFG = dict(TM=400, FC=512, KC=512, vmem_mb=120)

F32 = jnp.float32
BF16 = jnp.bfloat16
EPS = 1e-5


def _ln_scaled(x, post):
    mu = jnp.mean(x, axis=-1, keepdims=True)
    xc = x - mu
    var = jnp.mean(xc * xc, axis=-1, keepdims=True)
    inv = lax.rsqrt(var + EPS)
    if post != 1.0:
        inv = inv * post
    return xc * inv


def _dot(a, b):
    return jnp.dot(a, b, preferred_element_type=F32)


def _dot_nt(a, b):
    return lax.dot_general(a, b, (((1,), (1,)), ((), ())), preferred_element_type=F32)


def _ffn(h_half, wa_ref, wb_ref, FC):
    Fdim = wa_ref.shape[1]
    y = None
    for c in range(Fdim // FC):
        u = _dot(h_half, wa_ref[:, c * FC:(c + 1) * FC])
        a = (u + u * jnp.tanh(u)).astype(BF16)
        yc = _dot(a, wb_ref[c * FC:(c + 1) * FC, :])
        y = yc if y is None else y + yc
    return y


@jax.jit
def pallas_standalone__conformer_family_conformer__speech_kernel(
    x, w_ff1_a, w_ff1_b, w_q, w_k, w_v, w_o, w_pw1, dw, w_pw2, w_ff2_a, w_ff2_b,
):
    B, T, D = x.shape
    Fd = w_ff1_a.shape[1]
    K = dw.shape[0]
    TM, FC, KC = CFG['TM'], CFG['FC'], CFG['KC']
    NT = T // TM
    NTILES = B * NT
    TP = ((T + KC - 1) // KC) * KC
    NKC = TP // KC
    PAD = K // 2
    HALO = 8
    GROWS = T + 2 * HALO
    qscale = (D ** -0.5) * math.log2(math.e)

    def kernel(x_hbm, w1a_h, w1b_h, wq_h, wk_h, wv_h, wo_h, wp1_h, dw_h, wp2_h, w2a_h, w2b_h,
               o_hbm,
               xv, w1a, w1b, wq, wk, wv, wo, wp1, dwv, wp2, w2a, w2b,
               m_ref, wvo_ref, x1_ref, h_ref, s_ref, g_ref, dc_ref, st_ref, obuf,
               wsem, xsem, osem):
        wcopies = [
            pltpu.make_async_copy(s, d, wsem.at[i]) for i, (s, d) in enumerate([
                (wq_h, wq), (wk_h, wk), (w1a_h, w1a), (w1b_h, w1b), (wv_h, wv), (wo_h, wo),
                (wp1_h, wp1), (dw_h, dwv), (wp2_h, wp2), (w2a_h, w2a), (w2b_h, w2b)])]

        def xcopy(i):
            b, t = divmod(i, NT)
            return pltpu.make_async_copy(x_hbm.at[b, pl.ds(t * TM, TM)],
                                         xv.at[pl.ds(i * TM, TM)], xsem.at[i])

        xcopy(0).start()
        for c in wcopies[:4]:
            c.start()
        for i in range(1, NTILES):
            xcopy(i).start()
        for c in wcopies[4:]:
            c.start()

        for b in range(B):
            h_ref[b, T:TP, :] = jnp.zeros((TP - T, D), BF16)
            g_ref[b, 0:HALO, :] = jnp.zeros((HALO, D), F32)
            g_ref[b, HALO + T:GROWS, :] = jnp.zeros((HALO, D), F32)

        wcopies[0].wait()
        wcopies[1].wait()
        m_ref[...] = (_dot_nt(wq[...], wk[...]) * qscale).astype(BF16)
        wcopies[2].wait()
        wcopies[3].wait()

        def phase_a(i, carry):
            b = i // NT
            t = i - b * NT
            r0 = pl.multiple_of(i * TM, 16)
            pltpu.make_async_copy(x_hbm.at[b, pl.ds(t * TM, TM)],
                                  xv.at[pl.ds(r0, TM)], xsem.at[i]).wait()
            xt = xv[pl.ds(r0, TM), :].astype(F32)
            h = _ln_scaled(xt, 0.5).astype(BF16)
            y = _ffn(h, w1a, w1b, FC)
            x1 = xt + 0.5 * y
            x1_ref[pl.ds(r0, TM), :] = x1
            h_ref[b, pl.ds(pl.multiple_of(t * TM, 16), TM), :] = _ln_scaled(x1, 1.0).astype(BF16)
            return carry

        lax.fori_loop(0, NTILES, phase_a, 0)

        wcopies[4].wait()
        wcopies[5].wait()
        wvo_ref[...] = _dot(wv[...], wo[...]).astype(BF16)
        wcopies[6].wait()
        wcopies[7].wait()

        def phase_b(i, carry):
            b = i // NT
            t = i - b * NT
            r0 = pl.multiple_of(i * TM, 16)
            t0 = pl.multiple_of(t * TM, 16)
            hq = h_ref[b, pl.ds(t0, TM), :]
            q = _dot(hq, m_ref[...]).astype(BF16)
            mx = None
            for c in range(NKC):
                s = _dot_nt(q, h_ref[b, c * KC:(c + 1) * KC, :])
                if (c + 1) * KC > T:
                    col = lax.broadcasted_iota(jnp.int32, (TM, KC), 1)
                    s = jnp.where(col < T - c * KC, s, -jnp.inf)
                s_ref[:, c * KC:(c + 1) * KC] = s
                for j in range(KC // 128):
                    sj = s[:, j * 128:(j + 1) * 128]
                    mx = sj if mx is None else jnp.maximum(mx, sj)
            mrow = jnp.max(mx, axis=-1, keepdims=True)
            o = None
            ls = None
            for c in range(NKC):
                p = jnp.exp2(s_ref[:, c * KC:(c + 1) * KC] - mrow)
                for j in range(KC // 128):
                    pj = p[:, j * 128:(j + 1) * 128]
                    ls = pj if ls is None else ls + pj
                oc = _dot(p.astype(BF16), h_ref[b, c * KC:(c + 1) * KC, :])
                o = oc if o is None else o + oc
            lrow = jnp.sum(ls, axis=-1, keepdims=True)
            o = o * (1.0 / lrow)
            attn = _dot(o.astype(BF16), wvo_ref[...])
            x2 = x1_ref[pl.ds(r0, TM), :] + attn
            x1_ref[pl.ds(r0, TM), :] = x2
            h2 = _ln_scaled(x2, 1.0).astype(BF16)
            pw = _dot(h2, wp1[...])
            ga = pw[:, :D]
            gb = pw[:, D:]
            g = ga * (0.5 + 0.5 * jnp.tanh(0.5 * gb))
            g_ref[b, pl.ds(pl.multiple_of(t * TM + HALO, 8), TM), :] = g
            return carry

        lax.fori_loop(0, NTILES, phase_b, 0)

        dwf = dwv[...].astype(F32)

        def phase_conv(i, carry):
            b = i // NT
            t = i - b * NT
            r0 = pl.multiple_of(i * TM, 16)
            t0 = pl.multiple_of(t * TM, 16)
            acc = None
            win = g_ref[b, pl.ds(t0, TM + 2 * HALO), :]
            for k in range(K):
                off = HALO - PAD + k
                term = win[off:off + TM, :] * dwf[k:k + 1, :]
                acc = term if acc is None else acc + term
            dc_ref[pl.ds(r0, TM), :] = acc
            mean_i = jnp.sum(acc, axis=0, keepdims=True) * (1.0 / TM)
            dev = acc - mean_i
            m2_i = jnp.sum(dev * dev, axis=0, keepdims=True)
            mean, m2 = carry
            n_a = (i * TM).astype(F32)
            n_ab = n_a + TM
            delta = mean_i - mean
            mean_new = mean + delta * (TM / n_ab)
            m2_new = m2 + m2_i + delta * delta * (n_a * TM / n_ab)
            return mean_new, m2_new

        mean, m2 = lax.fori_loop(0, NTILES, phase_conv,
                                 (jnp.zeros((1, D), F32), jnp.zeros((1, D), F32)))
        bn_inv = lax.rsqrt(m2 * (1.0 / (B * T)) + EPS)

        wcopies[8].wait()
        wcopies[9].wait()
        wcopies[10].wait()

        def ocopy(i, slot):
            b = i // NT
            t = i - b * NT
            return pltpu.make_async_copy(obuf.at[slot], o_hbm.at[b, pl.ds(t * TM, TM)], osem.at[slot])

        def phase_c(i, carry):
            r0 = pl.multiple_of(i * TM, 16)
            slot = i % 2
            u = (dc_ref[pl.ds(r0, TM), :] - mean) * (0.5 * bn_inv)
            a = (u + u * jnp.tanh(u)).astype(BF16)
            x3 = x1_ref[pl.ds(r0, TM), :] + _dot(a, wp2[...])
            h = _ln_scaled(x3, 0.5).astype(BF16)
            y = _ffn(h, w2a, w2b, FC)
            x4 = x3 + 0.5 * y
            out = _ln_scaled(x4, 1.0).astype(BF16)

            @pl.when(i >= 2)
            def _():
                ocopy(i - 2, slot).wait()

            obuf[slot] = out
            ocopy(i, slot).start()
            return carry

        lax.fori_loop(0, NTILES, phase_c, 0)
        ocopy(NTILES - 2, (NTILES - 2) % 2).wait()
        ocopy(NTILES - 1, (NTILES - 1) % 2).wait()

    any_spec = pl.BlockSpec(memory_space=pl.ANY)
    scratch = [
        pltpu.VMEM((B * T, D), BF16),
        pltpu.VMEM((D, Fd), BF16), pltpu.VMEM((Fd, D), BF16),
        pltpu.VMEM((D, D), BF16), pltpu.VMEM((D, D), BF16), pltpu.VMEM((D, D), BF16), pltpu.VMEM((D, D), BF16),
        pltpu.VMEM((D, 2 * D), BF16), pltpu.VMEM((K, D), BF16), pltpu.VMEM((D, D), BF16),
        pltpu.VMEM((D, Fd), BF16), pltpu.VMEM((Fd, D), BF16),
        pltpu.VMEM((D, D), BF16), pltpu.VMEM((D, D), BF16),
        pltpu.VMEM((B * T, D), F32),
        pltpu.VMEM((B, TP, D), BF16),
        pltpu.VMEM((TM, TP), F32),
        pltpu.VMEM((B, GROWS, D), F32),
        pltpu.VMEM((B * T, D), F32),
        pltpu.VMEM((8, D), F32),
        pltpu.VMEM((2, TM, D), BF16),
        pltpu.SemaphoreType.DMA((11,)),
        pltpu.SemaphoreType.DMA((NTILES,)),
        pltpu.SemaphoreType.DMA((2,)),
    ]
    return pl.pallas_call(
        kernel,
        out_shape=jax.ShapeDtypeStruct((B, T, D), x.dtype),
        in_specs=[any_spec] * 12,
        out_specs=any_spec,
        scratch_shapes=scratch,
        compiler_params=pltpu.CompilerParams(vmem_limit_bytes=CFG['vmem_mb'] * 1024 * 1024),
    )(x, w_ff1_a, w_ff1_b, w_q, w_k, w_v, w_o, w_pw1, dw, w_pw2, w_ff2_a, w_ff2_b)
```

```python
import math
import numpy as np
import jax
import jax.numpy as jnp
from jax import lax
import jax.experimental.pallas as pl
import jax.experimental.pallas.tpu as pltpu

CFG = dict(TM=400, FC=512, KC=512, RB=40, vmem_mb=120, B_UNROLL=True, C_UNROLL=True, A_CARRY=True, flags={'XLA_TPU_EVENLY_DISTRIBUTE_CRITICAL_NODES': True}, B_SPLIT='dyn', ABL=None, CONV_IN_S=True, FORCE_S=False, EXP_NT=0, CONV_NT=2, FORCE_LAG=2, PACE_EXP=True, PACE_CONV=True, TIE_ALLW=False, TIE_STATS=True, STATS_TO='w', LAG=3, NPIECE=8, PPC=1, TIE_S=False)

F32 = jnp.float32
BF16 = jnp.bfloat16
EPS = 1e-5
LANES = 128


def _ln_scaled(x, post):
    mu = jnp.mean(x, axis=-1, keepdims=True)
    xc = x - mu
    var = jnp.mean(xc * xc, axis=-1, keepdims=True)
    inv = lax.rsqrt(var + EPS)
    if post != 1.0:
        inv = inv * post
    return xc * inv


def _dot(a, b):
    return jnp.dot(a, b, preferred_element_type=F32)


def _dot_nt(a, b):
    return lax.dot_general(a, b, (((1,), (1,)), ((), ())), preferred_element_type=F32)


def _zero_like_dep(on):
    return 0.0 * on


def _tie32(x, on):
    if on is None:
        return x
    top = x[0:8, 0:LANES] + _zero_like_dep(on)
    row0 = jnp.concatenate([top, x[0:8, LANES:]], axis=1) if x.shape[1] > LANES else top
    return jnp.concatenate([row0, x[8:, :]], axis=0)


def _tie_bf16(x32, xb, on):
    if on is None:
        return xb
    z = _zero_like_dep(on)
    top = jnp.concatenate([x32[0:8, 0:LANES] + z, x32[8:16, 0:LANES] + z], axis=0).astype(BF16)
    row0 = jnp.concatenate([top, xb[0:16, LANES:]], axis=1)
    return jnp.concatenate([row0, xb[16:, :]], axis=0)


def _ffn(h_half, wa_ref, wb_ref, FC):
    Fdim = wa_ref.shape[1]
    y = None
    for c in range(Fdim // FC):
        u = _dot(h_half, wa_ref[:, c * FC:(c + 1) * FC])
        a = (u + u * jnp.tanh(u)).astype(BF16)
        yc = _dot(a, wb_ref[c * FC:(c + 1) * FC, :])
        y = yc if y is None else y + yc
    return y


@jax.jit
def pallas_standalone__conformer_family_conformer__speech_kernel(
    x, w_ff1_a, w_ff1_b, w_q, w_k, w_v, w_o, w_pw1, dw, w_pw2, w_ff2_a, w_ff2_b,
):
    B, T, D = x.shape
    Fd = w_ff1_a.shape[1]
    K = dw.shape[0]
    TM, FC, KC, RB = CFG['TM'], CFG['FC'], CFG['KC'], CFG['RB']
    NT = T // TM
    N = B * NT
    TP = ((T + KC - 1) // KC) * KC
    NKC = TP // KC
    PAD = K // 2
    HALO = 8
    GROWS = T + 2 * HALO
    NCC = D // LANES
    qscale = (D ** -0.5) * math.log2(math.e)

    def rows(i):
        return pl.ds(pl.multiple_of(i * TM, 16), TM)

    def kernel(x_hbm, w1a_h, w1b_h, wq_h, wk_h, wv_h, wo_h, wp1_h, dw_h, wp2_h, w2a_h, w2b_h,
               o_hbm,
               xv, w1a, w1b, wq, wk, wv, wo, wp1, dwv, wp2, w2a, w2b,
               m_ref, wvo_ref, x1_ref, h_ref, s2, g_ref, dc_ref, st_ref,
               hc_a, hc_b, x3_a, x3_b, mr2,
               wsem, xsem, osem):
        s_a, s_b, mr_a, mr_b = s2.at[0], s2.at[1], mr2.at[0], mr2.at[1]

        srcs = [wq_h, wk_h, wv_h, wo_h, w1a_h, w1b_h, wp1_h, dw_h, wp2_h, w2a_h, w2b_h]
        dsts = [wq, wk, wv, wo, w1a, w1b, wp1, dwv, wp2, w2a, w2b]
        wcp = [pltpu.make_async_copy(s, d, wsem.at[i]) for i, (s, d) in enumerate(zip(srcs, dsts))]
        WQ, WK, WV, WO, W1A, W1B, WP1, DW, WP2, W2A, W2B = range(11)

        def xcopy(i):
            b = i // NT
            t = i - b * NT
            return pltpu.make_async_copy(x_hbm.at[b, pl.ds(t * TM, TM)], xv.at[rows(i)], xsem.at[i])

        for k in (WQ, WK):
            wcp[k].start()
        xcopy(0).start()
        wcp[W1A].start()
        wcp[W1B].start()
        xcopy(1).start()
        wcp[WV].start()
        wcp[WO].start()

        zrow = jnp.zeros((HALO, LANES), F32)
        for b in range(B):
            h_ref[b, T:TP, :] = jnp.zeros((TP - T, D), BF16)
            for cc in range(NCC):
                g_ref[b, cc, 0:HALO, :] = zrow
                g_ref[b, cc, HALO + T:GROWS, :] = zrow
        for cc in range(NCC):
            g_ref[0, cc, HALO:2 * HALO + TM, :] = jnp.zeros((TM + HALO, LANES), F32)
        x1_ref[0:TM, :] = jnp.zeros((TM, D), F32)

        wcp[WQ].wait()
        wcp[WK].wait()
        m_ref[...] = (_dot_nt(wq[...], wk[...]) * qscale).astype(BF16)

        xcopy(0).wait()
        h0 = _ln_scaled(xv[0:TM, :].astype(F32), 0.5).astype(BF16)
        wcp[W1A].wait()
        wcp[W1B].wait()
        for i in range(2, N):
            xcopy(i).start()
        for k in (WP1, DW, WP2, W2A, W2B):
            wcp[k].start()

        def h1_store(i):
            b = i // NT
            t = i - b * NT
            h_ref[b, pl.ds(pl.multiple_of(t * TM, 16), TM), :] = (
                _ln_scaled(x1_ref[rows(i), :], 1.0).astype(BF16))

        def phase_a(i, hcur):
            @pl.when(i + 1 < N)
            def _():
                xcopy(i + 1).wait()

            h1_store(jnp.maximum(i - 1, 0))
            inext = jnp.minimum(i + 1, N - 1)
            hnext = _ln_scaled(xv[rows(inext), :].astype(F32), 0.5).astype(BF16)
            y = _ffn(hcur, w1a, w1b, FC)
            x1_ref[rows(i), :] = xv[rows(i), :].astype(F32) + 0.5 * y
            return hnext

        with jax.named_scope('s1_phaseA'):
            lax.fori_loop(0, N, phase_a, h0)

        wcp[WV].wait()
        wcp[WO].wait()
        wvo_ref[...] = _dot(wv[...], wo[...]).astype(BF16)
        h1_store(N - 1)
        wcp[WP1].wait()
        wcp[DW].wait()

        def q_proj(i):
            b = i // NT
            t = i - b * NT
            hq = h_ref[b, pl.ds(pl.multiple_of(t * TM, 16), TM), :]
            q32 = _dot(hq, m_ref[...])
            return q32[0:16, 0:LANES], q32.astype(BF16)

        def score_chunk(i, c, q, s_ref, mx, end_tie=None):
            b = i // NT
            s = _dot_nt(q, h_ref[b, c * KC:(c + 1) * KC, :])
            if (c + 1) * KC > T:
                col = lax.broadcasted_iota(jnp.int32, (TM, KC), 1)
                s = jnp.where(col < T - c * KC, s, -jnp.inf)
            s_ref[:, c * KC:(c + 1) * KC] = s
            for j in range(KC // LANES):
                sj = s[:, j * LANES:(j + 1) * LANES]
                mx = sj if mx is None else jnp.maximum(mx, sj)
            if end_tie is not None:
                mx = _tie32(mx, end_tie)
            return mx, s

        def pv_chunk(i, c, s_ref, mrow_b, o, ls, tie=None, pace=None):
            b = i // NT
            if pace is not None:
                mrow_b = mrow_b + _zero_like_dep(pace)
            p = jnp.exp2(s_ref[:, c * KC:(c + 1) * KC] - jnp.concatenate([mrow_b] * (KC // LANES), axis=1))
            for j in range(KC // LANES):
                pj = p[:, j * LANES:(j + 1) * LANES]
                ls = pj if ls is None else ls + pj
            p = _tie32(p, tie)
            oc = _dot(p.astype(BF16), h_ref[b, c * KC:(c + 1) * KC, :])
            return (oc if o is None else o + oc), ls, oc

        def out_proj(i, o, ls, tie=None):
            lrow = jnp.sum(ls, axis=-1, keepdims=True)
            o = _tie32(o * (1.0 / lrow), tie)
            attn = _dot(o.astype(BF16), wvo_ref[...])
            x2 = x1_ref[rows(i), :] + attn
            x1_ref[rows(i), :] = x2
            return x2, attn[0:8, 0:LANES]

        def glu(i, x2, tie=None):
            b = i // NT
            t = i - b * NT
            h2 = _tie32(_ln_scaled(x2, 1.0), tie).astype(BF16)
            pw = _dot(h2, wp1[...])
            g = pw[:, :D] * (0.5 + 0.5 * jnp.tanh(0.5 * pw[:, D:]))
            for cc in range(NCC):
                g_ref[b, cc, pl.ds(pl.multiple_of(t * TM + HALO, 8), TM), :] = (
                    g[:, cc * LANES:(cc + 1) * LANES])
            return pw[0:8, 0:LANES]

        NPIECE = CFG['NPIECE']
        RP = NPIECE // NCC
        RROWS = TM // RP

        def conv_piece(i, k, pace=None):
            b = i // NT
            t = i - b * NT
            t0 = pl.multiple_of(t * TM, 16)
            r0 = pl.multiple_of(i * TM, 16)
            cc, rp = divmod(k, RP)
            dwf = dwv[:, cc * LANES:(cc + 1) * LANES].astype(F32)
            w1 = [jnp.broadcast_to(dwf[kk:kk + 1, :], (8, LANES)) for kk in range(K)]
            ssum = None
            nblk = RROWS // RB
            for rb in range(nblk):
                w = list(w1)
                if pace is not None:
                    pr = (pace.shape[0] // 8 * rb // nblk) * 8
                    z = _zero_like_dep(pace[pr:pr + 8, :])
                    w = [wk + z for wk in w] if CFG['TIE_ALLW'] else [w[0] + z] + w[1:]
                w = [jnp.concatenate([wk] * (RB // 8), axis=0) for wk in w]
                off = rp * RROWS + rb * RB
                acc = None
                for kk in range(K):
                    v = g_ref[b, cc, pl.ds(t0 + (off + HALO - PAD + kk), RB), :]
                    term = v * w[kk]
                    acc = term if acc is None else acc + term
                dc_ref[pl.ds(pl.multiple_of(r0 + off, 8), RB), cc * LANES:(cc + 1) * LANES] = acc
                for j in range(RB // 8):
                    aj = acc[j * 8:(j + 1) * 8, :]
                    ssum = aj if ssum is None else ssum + aj
            return ssum

        def conv_stats(i, sums, start_tie=None):
            r0 = pl.multiple_of(i * TM, 16)
            cols = []
            for cc in range(NCC):
                sc = sums[cc * RP]
                for rp in range(1, RP):
                    sc = sc + sums[cc * RP + rp]
                if start_tie is not None:
                    sc = sc + _zero_like_dep(start_tie)
                cols.append(jnp.sum(sc, axis=0, keepdims=True))
            mean_i = jnp.concatenate(cols, axis=1) * (1.0 / TM)
            dev = dc_ref[pl.ds(r0, TM), :] - mean_i
            m2_i = jnp.sum(dev * dev, axis=0, keepdims=True)
            st_ref[i, 0:1, :] = mean_i
            st_ref[i, 1:2, :] = m2_i
            return jnp.broadcast_to(m2_i[:, 0:LANES], (8, LANES))

        def conv(i):
            sums = [conv_piece(i, k) for k in range(NPIECE)]
            conv_stats(i, sums)

        def step(inext, s_next, icur, s_cur, mx_cur, iconv):
            LAG = CFG['LAG'] if (inext is not None and icur is not None) else 0
            q32 = q = qfull = None
            if inext is not None:
                b = inext // NT
                t = inext - b * NT
                hq = h_ref[b, pl.ds(pl.multiple_of(t * TM, 16), TM), :]
                qfull = _dot(hq, m_ref[...])
                q32 = qfull[0:16, 0:LANES]
                q = qfull.astype(BF16)
            mx = o = ls = None
            sums = []
            if icur is not None:
                mrow_b = jnp.broadcast_to(jnp.max(mx_cur, axis=-1, keepdims=True), (TM, LANES))
                EN, CN = CFG['EXP_NT'], CFG['CONV_NT']
                FL = CFG['FORCE_LAG']
                conv_in_s = CFG['CONV_IN_S'] and inext is not None
                ocs = [qfull]
                for c in range(NKC):
                    prev = ocs[c]
                    pace = prev[:, EN * LANES:(EN + 1) * LANES] if (prev is not None and CFG['PACE_EXP']) else None
                    tie = None
                    if iconv is not None and not conv_in_s:
                        if c < NPIECE:
                            cpace = prev[:, CN * LANES:(CN + 1) * LANES] if (prev is not None and CFG['PACE_CONV']) else None
                            sums.append(conv_piece(iconv, c, cpace))
                        tie = sums[c - FL] if c - FL >= 0 else None
                    o, ls, oc = pv_chunk(icur, c, s_cur, mrow_b, o, ls, tie, pace)
                    ocs.append(oc)
                last_started = ocs[-1][0:8, 0:LANES]
                order = ['pv', 'o', 'w'][3 - LAG:] if LAG else []
                sidx = NKC - LAG
                sres = None
                stats_pace = last_started
                if inext is not None:
                    nfree = NKC - LAG
                    prev_s = None
                    for c in range(nfree):
                        qq = q
                        if conv_in_s and iconv is not None and CFG['FORCE_S'] and c >= FL + 1:
                            k0, k1 = (c - FL - 1) * NPIECE // nfree, (c - FL) * NPIECE // nfree
                            if k1 > k0:
                                tt = sums[k0]
                                for k in range(k0 + 1, k1):
                                    tt = tt + sums[k]
                                qq = _tie_bf16(q32, q, tt)
                        mx, sfull = score_chunk(inext, c, qq, s_next, mx)
                        if conv_in_s and iconv is not None:
                            k0, k1 = c * NPIECE // nfree, (c + 1) * NPIECE // nfree
                            for k in range(k0, k1):
                                nt = (CN + k - k0) % (KC // LANES)
                                sums.append(conv_piece(iconv, k, sfull[:, nt * LANES:(nt + 1) * LANES]))
                        stats_pace = sfull[TM - 8:TM, (KC - LANES):KC]
                    if 'pv' in order:
                        mx, _ = score_chunk(inext, sidx, _tie_bf16(q32, q, last_started), s_next, mx)
                        sidx += 1
                tie = None
                if iconv is not None:
                    for c in range(0 if conv_in_s else max(NKC - FL, 0), NPIECE):
                        tie = sums[c] if tie is None else tie + sums[c]
                tie_stats = conv_stats(iconv, sums, stats_pace if CFG['TIE_STATS'] else None) if iconv is not None else None
                x2, o_started = out_proj(icur, o, ls, tie)
                if inext is not None and 'o' in order:
                    mx, _ = score_chunk(inext, sidx, _tie_bf16(q32, q, o_started), s_next, mx)
                    sidx += 1
                w_started = glu(icur, x2, tie_stats if CFG['STATS_TO'] == 'w' else None)
                if inext is not None and 'w' in order:
                    qq = _tie_bf16(q32, q, w_started)
                    mx, _ = score_chunk(inext, sidx, qq, s_next, mx, tie_stats if CFG['STATS_TO'] == 's' else None)
                    sidx += 1
            else:
                for c in range(NKC):
                    mx, _ = score_chunk(inext, c, q, s_next, mx)
            return mx

        with jax.named_scope('s2_Bpro'):
            mr_a[...] = step(0, s_a, None, None, None, None)

        if CFG['B_SPLIT'] == 'dyn':
            def phase_b(i, carry):
                ic = jnp.maximum(i - 2, 0)
                cur = i % 2
                nxt = 1 - cur
                mr2[nxt] = step(i + 1, s2.at[nxt], i, s2.at[cur], mr2[cur], None if CFG['ABL'] == 'noconv' else ic)
                return carry

            with jax.named_scope('s3_phaseB'):
                lax.fori_loop(0, N - 2, phase_b, 0)
        elif CFG['B_SPLIT']:
            def phase_b(i, carry):
                ic = jnp.maximum(i - 2, 0)

                @pl.when(i % 2 == 0)
                def _():
                    mr_b[...] = step(i + 1, s_b, i, s_a, mr_a[...], ic)

                @pl.when(i % 2 == 1)
                def _():
                    mr_a[...] = step(i + 1, s_a, i, s_b, mr_b[...], ic)
                return carry

            with jax.named_scope('s3_phaseB'):
                lax.fori_loop(0, N - 2, phase_b, 0)
        else:
            def phase_b(j, carry):
                i = 2 * j
                mr_b[...] = step(i + 1, s_b, i, s_a, mr_a[...], jnp.maximum(i - 2, 0))
                mr_a[...] = step(i + 2, s_a, i + 1, s_b, mr_b[...], jnp.maximum(i - 1, 0))
                return carry

            with jax.named_scope('s3_phaseB'):
                lax.fori_loop(0, N // 2 - 1, phase_b, 0)
        with jax.named_scope('s4_Bepi'):
            mr_b[...] = step(N - 1, s_b, N - 2, s_a, mr_a[...], N - 4)
            step(None, None, N - 1, s_b, mr_b[...], N - 3)
        with jax.named_scope('s5_conv'):
            conv(N - 2)
            conv(N - 1)

        means = st_ref[:, 0, :]
        m2s = st_ref[:, 1, :]
        mean = jnp.mean(means, axis=0, keepdims=True)
        dm = means - mean
        m2 = jnp.sum(m2s + dm * dm * float(TM), axis=0, keepdims=True)
        bn_scale = 0.5 * lax.rsqrt(m2 * (1.0 / (B * T)) + EPS)

        wcp[WP2].wait()
        wcp[W2A].wait()
        wcp[W2B].wait()

        def ocopy(i):
            b = i // NT
            t = i - b * NT
            return pltpu.make_async_copy(xv.at[rows(i)], o_hbm.at[b, pl.ds(t * TM, TM)], osem.at[i])

        def pre(i, x3_ref, hc_ref):
            u = (dc_ref[rows(i), :] - mean) * bn_scale
            a = (u + u * jnp.tanh(u)).astype(BF16)
            x3 = x1_ref[rows(i), :] + _dot(a, wp2[...])
            x3_ref[...] = x3
            hc_ref[...] = _ln_scaled(x3, 0.5).astype(BF16)

        def ffn2(i, x3_ref, hc_ref):
            y = _ffn(hc_ref[...], w2a, w2b, FC)
            x1_ref[rows(i), :] = x3_ref[...] + 0.5 * y

        def post(i):
            xv[rows(i), :] = _ln_scaled(x1_ref[rows(i), :], 1.0).astype(BF16)

        with jax.named_scope('s6_Cpro'):
            pre(0, x3_a, hc_a)

        def phase_c(j, carry):
            i = 2 * j
            pre(i + 1, x3_b, hc_b)
            post(jnp.maximum(i - 1, 0))
            ffn2(i, x3_a, hc_a)
            post(i)
            pre(jnp.minimum(i + 2, N - 1), x3_a, hc_a)
            ffn2(i + 1, x3_b, hc_b)

            @pl.when(j > 0)
            def _():
                ocopy(i - 1).start()
            ocopy(i).start()
            return carry

        with jax.named_scope('s7_phaseC'):
            lax.fori_loop(0, N // 2, phase_c, 0)
        with jax.named_scope('s8_tail'):
            post(N - 1)
            ocopy(N - 1).start()
            for i in range(N):
                ocopy(i).wait()

    any_spec = pl.BlockSpec(memory_space=pl.ANY)
    scratch = [
        pltpu.VMEM((B * T, D), BF16),
        pltpu.VMEM((D, Fd), BF16), pltpu.VMEM((Fd, D), BF16),
        pltpu.VMEM((D, D), BF16), pltpu.VMEM((D, D), BF16), pltpu.VMEM((D, D), BF16), pltpu.VMEM((D, D), BF16),
        pltpu.VMEM((D, 2 * D), BF16), pltpu.VMEM((K, D), BF16), pltpu.VMEM((D, D), BF16),
        pltpu.VMEM((D, Fd), BF16), pltpu.VMEM((Fd, D), BF16),
        pltpu.VMEM((D, D), BF16), pltpu.VMEM((D, D), BF16),
        pltpu.VMEM((B * T, D), F32),
        pltpu.VMEM((B, TP, D), BF16),
        pltpu.VMEM((2, TM, TP), F32),
        pltpu.VMEM((B, NCC, GROWS, LANES), F32),
        pltpu.VMEM((B * T, D), F32),
        pltpu.VMEM((N, 8, D), F32),
        pltpu.VMEM((TM, D), BF16), pltpu.VMEM((TM, D), BF16),
        pltpu.VMEM((TM, D), F32), pltpu.VMEM((TM, D), F32),
        pltpu.VMEM((2, TM, LANES), F32),
        pltpu.SemaphoreType.DMA((11,)),
        pltpu.SemaphoreType.DMA((N,)),
        pltpu.SemaphoreType.DMA((N,)),
    ]
    return pl.pallas_call(
        kernel,
        out_shape=jax.ShapeDtypeStruct((B, T, D), x.dtype),
        in_specs=[any_spec] * 12,
        out_specs=any_spec,
        scratch_shapes=scratch,
        compiler_params=pltpu.CompilerParams(vmem_limit_bytes=CFG['vmem_mb'] * 1024 * 1024, flags=CFG.get('flags')),
    )(x, w_ff1_a, w_ff1_b, w_q, w_k, w_v, w_o, w_pw1, dw, w_pw2, w_ff2_a, w_ff2_b)
```

```python
import math
import numpy as np
import jax
import jax.numpy as jnp
from jax import lax
import jax.experimental.pallas as pl
import jax.experimental.pallas.tpu as pltpu

CFG = dict(TM=400, FC=512, KC=512, RB=40, vmem_mb=120,
           flags={'XLA_TPU_EVENLY_DISTRIBUTE_CRITICAL_NODES': True},
           LAG=3, NPIECE=8, EXP_NT=0, CONV_NT=2, POLY=True, FPOLY=False, OLDC=False, SPAD=0, A_CARRY=False, A_PACE=(1, 2), C_PACE=(0, 1, 2), ABL='', NCV=6, CONV_FORCE='s7', STATS_FORCE='end', STATS_START=True, SCOPES=False,
           A_TIES=False, C_TIES=False)

F32 = jnp.float32
BF16 = jnp.bfloat16
EPS = 1e-5
LANES = 128


def _ln_scaled(x, post):
    mu = jnp.mean(x, axis=-1, keepdims=True)
    xc = x - mu
    var = jnp.mean(xc * xc, axis=-1, keepdims=True)
    inv = lax.rsqrt(var + EPS)
    if post != 1.0:
        inv = inv * post
    return xc * inv


def _dot(a, b):
    return jnp.dot(a, b, preferred_element_type=F32)


def _dot_nt(a, b):
    return lax.dot_general(a, b, (((1,), (1,)), ((), ())), preferred_element_type=F32)


def _tie32(x, on):
    if on is None:
        return x
    top = x[0:8, 0:LANES] + 0.0 * on
    row0 = jnp.concatenate([top, x[0:8, LANES:]], axis=1) if x.shape[1] > LANES else top
    return jnp.concatenate([row0, x[8:, :]], axis=0)


def _tie_bf16(x32, xb, on):
    if on is None:
        return xb
    z = 0.0 * on
    top = jnp.concatenate([x32[0:8, :] + z, x32[8:16, :] + z], axis=0).astype(BF16)
    row0 = jnp.concatenate([top, xb[0:16, LANES:]], axis=1)
    return jnp.concatenate([row0, xb[16:, :]], axis=0)


def _spread(res):
    nr = res.shape[0] // 8
    nt = res.shape[1] // LANES
    out = []
    for r in range(nr):
        j, rr = divmod(r * nt, nr)
        out.append(res[rr * 8:(rr + 1) * 8, j * LANES:(j + 1) * LANES])
    return jnp.concatenate(out, axis=0)


def _pace_rows(x, res):
    if res is None:
        return x
    left = x[:, 0:LANES] + 0.0 * _spread(res)
    return jnp.concatenate([left, x[:, LANES:]], axis=1)


def _silu_half(u):
    return u + u * jnp.tanh(u)


class _Scope:
    def __init__(self, name):
        self.cm = jax.named_scope(name) if CFG['SCOPES'] else None

    def __enter__(self):
        if self.cm is not None:
            self.cm.__enter__()

    def __exit__(self, *a):
        if self.cm is not None:
            self.cm.__exit__(*a)


@jax.jit
def pallas_standalone__conformer_family_conformer__speech_kernel(
    x, w_ff1_a, w_ff1_b, w_q, w_k, w_v, w_o, w_pw1, dw, w_pw2, w_ff2_a, w_ff2_b,
):
    B, T, D = x.shape
    Fd = w_ff1_a.shape[1]
    K = dw.shape[0]
    TM, FC, KC, RB = CFG['TM'], CFG['FC'], CFG['KC'], CFG['RB']
    NT = T // TM
    N = B * NT
    NFC = Fd // FC
    TP = ((T + KC - 1) // KC) * KC
    NKC = TP // KC
    PAD = K // 2
    HALO = 8
    GROWS = T + 2 * HALO
    NCC = D // LANES
    NBLK = TM // RB
    qscale = (D ** -0.5) * math.log2(math.e)

    def rows(i):
        return pl.ds(pl.multiple_of(i * TM, 16), TM)

    def bt(i):
        b = i // NT
        return b, pl.multiple_of((i - b * NT) * TM, 16)

    def kernel(x_hbm, w1a_h, w1b_h, wq_h, wk_h, wv_h, wo_h, wp1_h, dw_h, wp2_h, w2a_h, w2b_h,
               o_hbm,
               xv, w1a, w1b, wq, wk, wv, wo, wp1, dwv, wp2, w2a, w2b,
               m_ref, wvo_ref, x1_ref, h_ref, s2, g_ref, dc_ref, st_ref,
               hc_a, hc_b, x3_a, x3_b, mr2, hbuf,
               wsem, csem, xsem, osem):
        srcs = [wq_h, wk_h, wv_h, wo_h, wp1_h, dw_h, wp2_h, w2a_h, w2b_h]
        dsts = [wq, wk, wv, wo, wp1, dwv, wp2, w2a, w2b]
        wcp = [pltpu.make_async_copy(s, d, wsem.at[i]) for i, (s, d) in enumerate(zip(srcs, dsts))]
        WQ, WK, WV, WO, WP1, DW, WP2, W2A, W2B = range(9)
        acp = [pltpu.make_async_copy(w1a_h.at[:, pl.ds(c * FC, FC)], w1a.at[:, pl.ds(c * FC, FC)], csem.at[c])
               for c in range(NFC)]
        bcp = [pltpu.make_async_copy(w1b_h.at[pl.ds(c * FC, FC)], w1b.at[pl.ds(c * FC, FC)], csem.at[NFC + c])
               for c in range(NFC)]

        def xcopy(i):
            b, t0 = bt(i)
            return pltpu.make_async_copy(x_hbm.at[b, pl.ds(t0, TM)], xv.at[rows(i)], xsem.at[i])

        xcopy(0).start()
        acp[0].start()
        bcp[0].start()

        zrow = jnp.zeros((HALO, LANES), F32)
        for b in range(B):
            h_ref[b, T:TP, :] = jnp.zeros((TP - T, D), BF16)
            for cc in range(NCC):
                g_ref[b, cc, 0:HALO, :] = zrow
                g_ref[b, cc, HALO + T:GROWS, :] = zrow
        for cc in range(NCC):
            g_ref[0, cc, HALO:2 * HALO + TM, :] = jnp.zeros((TM + HALO, LANES), F32)

        def ffn(h_half, wa_ref, wb_ref, before_chunk=None, hooks=None):
            y = None
            for c in range(NFC):
                if before_chunk is not None:
                    before_chunk(c)
                u = _dot(h_half, wa_ref[:, c * FC:(c + 1) * FC])
                if hooks is not None and hooks.get(c) is not None:
                    hooks[c](u)
                a = _silu_half(u).astype(BF16)
                yc = _dot(a, wb_ref[c * FC:(c + 1) * FC, :])
                y = yc if y is None else y + yc
            return y

        def ln_in(i, pace=None):
            return _ln_scaled(_pace_rows(xv[rows(i), :].astype(F32), pace), 0.5).astype(BF16)

        def h1_store(i, pace=None):
            b, t0 = bt(i)
            h_ref[b, pl.ds(t0, TM), :] = _ln_scaled(_pace_rows(x1_ref[rows(i), :], pace), 1.0).astype(BF16)

        with _Scope('s0_first'):
            xcopy(0).wait()
            acp[1].start()
            bcp[1].start()
            h0 = ln_in(0)

            def wait_chunk(c):
                acp[c].wait()
                bcp[c].wait()
                if c + 2 < NFC:
                    acp[c + 2].start()
                    bcp[c + 2].start()
                if c == NFC - 3:
                    xcopy(1).start()
                    xcopy(2).start()
                if c == NFC - 2:
                    for k in (WQ, WK, WV, WO):
                        wcp[k].start()
                if c == NFC - 1:
                    for i in range(3, N):
                        xcopy(i).start()
                    for k in (WP1, DW, WP2, W2A, W2B):
                        wcp[k].start()

            y0 = ffn(h0, w1a, w1b, wait_chunk)
            x1_ref[0:TM, :] = xv[0:TM, :].astype(F32) + 0.5 * y0
            xcopy(1).wait()
            hbuf[1] = ln_in(1)

        def phase_a(i, carry):
            @pl.when(i + 1 < N)
            def _():
                xcopy(i + 1).wait()

            cur = i % 2
            P0, P1 = CFG['A_PACE']
            box = {}

            def next_h(u):
                hn = ln_in(jnp.minimum(i + 1, N - 1), u)
                if CFG['A_CARRY']:
                    box['h'] = hn
                else:
                    hbuf[1 - cur] = hn

            hooks = {}
            if P0 is None:
                next_h(None)
            else:
                hooks[P0] = next_h
            if P1 is None:
                h1_store(i - 1)
            else:
                hooks[P1] = lambda u: h1_store(i - 1, u)
            y = ffn(carry if CFG['A_CARRY'] else hbuf[cur], w1a, w1b, hooks=hooks)
            x1_ref[rows(i), :] = xv[rows(i), :].astype(F32) + 0.5 * y
            return box['h'] if CFG['A_CARRY'] else carry

        with _Scope('s1_phaseA'):
            lax.fori_loop(1, N, phase_a, hbuf[1] if CFG['A_CARRY'] else 0)

        with _Scope('s1b_fold'):
            for k in (WQ, WK, WV, WO):
                wcp[k].wait()
            m_ref[...] = (_dot_nt(wq[...], wk[...]) * qscale).astype(BF16)
            wvo_ref[...] = _dot(wv[...], wo[...]).astype(BF16)
            h1_store(N - 1)
            wcp[WP1].wait()
            wcp[DW].wait()

        def score_chunk(i, c, q, s_ref, mx):
            b = i // NT
            s = _dot_nt(q, h_ref[b, c * KC:(c + 1) * KC, :])
            if (c + 1) * KC > T:
                col = lax.broadcasted_iota(jnp.int32, (TM, KC), 1)
                s = jnp.where(col < T - c * KC, s, -jnp.inf)
            s_ref[:, c * KC:(c + 1) * KC] = s
            for j in range(KC // LANES):
                sj = s[:, j * LANES:(j + 1) * LANES]
                mx = sj if mx is None else jnp.maximum(mx, sj)
            return mx, s

        def pv_chunk(i, c, s_ref, mrow_b, o, ls, pace=None):
            b = i // NT
            if pace is not None:
                mrow_b = mrow_b + 0.0 * pace
            p = s_ref[:, c * KC:(c + 1) * KC] - jnp.concatenate([mrow_b] * (KC // LANES), axis=1)
            p = p if 'noexp' in CFG['ABL'] else jnp.exp2(p)
            for j in range(KC // LANES):
                pj = p[:, j * LANES:(j + 1) * LANES]
                ls = pj if ls is None else ls + pj
            oc = _dot(p.astype(BF16), h_ref[b, c * KC:(c + 1) * KC, :])
            return (oc if o is None else o + oc), ls, oc

        def out_proj(i, o, ls, tie=None):
            lrow = jnp.sum(ls, axis=-1, keepdims=True)
            o = _tie32(o * (1.0 / lrow), tie)
            attn = _dot(o.astype(BF16), wvo_ref[...])
            x2 = x1_ref[rows(i), :] + attn
            x1_ref[rows(i), :] = x2
            return x2, attn[0:8, 0:LANES]

        def glu(i, x2, tie=None):
            b, t0 = bt(i)
            h2 = _tie32(_ln_scaled(x2, 1.0), tie).astype(BF16)
            pw = _dot(h2, wp1[...])
            g = pw[:, :D] * (0.5 + 0.5 * jnp.tanh(0.5 * pw[:, D:]))
            for cc in range(NCC):
                g_ref[b, cc, pl.ds(pl.multiple_of(t0 + HALO, 8), TM), :] = g[:, cc * LANES:(cc + 1) * LANES]
            return pw[0:8, 0:LANES]

        def conv_block(i, k, pace=None, poly=None):
            b, t0 = bt(i)
            r0 = pl.multiple_of(i * TM, 16)
            cc, rb = divmod(k, NBLK)
            poly = CFG['POLY'] if poly is None else poly
            off = rb * RB
            dwf = dwv[:, cc * LANES:(cc + 1) * LANES].astype(F32)
            w = [jnp.broadcast_to(dwf[kk:kk + 1, :], (8, LANES)) for kk in range(K)]
            if pace is not None:
                z = 0.0 * pace
                w = [wk + z for wk in w] if poly else [w[0] + z] + w[1:]
            if poly:
                wt = [jnp.concatenate([wk] * (RB // 8 + 1), axis=0) for wk in w]
                ga = [g_ref[b, cc, pl.ds(pl.multiple_of(t0 + (off + 8 * a), 8), RB + 8), :] for a in range(2)]
                acc = None
                for sft in range(8):
                    zs = None
                    for a in range(2):
                        kk = 8 * a + sft - (HALO - PAD)
                        if 0 <= kk < K:
                            term = ga[a] * wt[kk]
                            zs = term if zs is None else zs + term
                    part = zs[sft:sft + RB, :]
                    acc = part if acc is None else acc + part
            else:
                wt = [jnp.concatenate([wk] * (RB // 8), axis=0) for wk in w]
                acc = None
                for kk in range(K):
                    if 'aligned' in CFG['ABL']:
                        v = g_ref[b, cc, pl.ds(pl.multiple_of(t0 + (off + 8 * kk), 8), RB), :] if False else g_ref[b, cc, pl.ds(pl.multiple_of(t0 + (off + 8 * (kk % 3)), 8), RB), :] + float(kk)
                    else:
                        v = g_ref[b, cc, pl.ds(t0 + (off + HALO - PAD + kk), RB), :]
                    term = v * wt[kk]
                    acc = term if acc is None else acc + term
            dc_ref[pl.ds(pl.multiple_of(r0 + off, 8), RB), cc * LANES:(cc + 1) * LANES] = acc
            ssum = None
            for j in range(RB // 8):
                aj = acc[j * 8:(j + 1) * 8, :]
                ssum = aj if ssum is None else ssum + aj
            return ssum

        def conv_paced(i, c, nchunks, res):
            nb = NCC * NBLK
            k0, k1 = c * nb // nchunks, (c + 1) * nb // nchunks
            out = []
            npass = res.shape[1] // LANES
            for k in range(k0, k1):
                pos = (k - k0) * npass * (TM // 8) // (k1 - k0)
                nt, r = divmod(pos, TM // 8)
                out.append(conv_block(i, k, res[r * 8:(r + 1) * 8, nt * LANES:(nt + 1) * LANES]))
            return out

        def conv_stats(i, sums, start_tie=None):
            r0 = pl.multiple_of(i * TM, 16)
            cols = []
            for cc in range(NCC):
                sc = sums[cc * NBLK]
                for rb in range(1, NBLK):
                    sc = sc + sums[cc * NBLK + rb]
                if start_tie is not None:
                    sc = sc + 0.0 * start_tie
                cols.append(jnp.sum(sc, axis=0, keepdims=True))
            mean_i = jnp.concatenate(cols, axis=1) * (1.0 / TM)
            dev = dc_ref[pl.ds(r0, TM), :] - mean_i
            m2_i = jnp.sum(dev * dev, axis=0, keepdims=True)
            st_ref[i, 0:1, :] = mean_i
            st_ref[i, 1:2, :] = m2_i
            return jnp.broadcast_to(m2_i[:, 0:LANES], (8, LANES))

        def conv(i):
            conv_stats(i, [conv_block(i, k, poly=CFG['FPOLY']) for k in range(NCC * NBLK)])

        def step(inext, s_next, icur, s_cur, mx_cur, iconv):
            LAG = CFG['LAG'] if (inext is not None and icur is not None) else 0
            q32 = q = qfull = None
            if inext is not None:
                b, t0 = bt(inext)
                qfull = _dot(h_ref[b, pl.ds(t0, TM), :], m_ref[...])
                q32 = qfull[0:16, 0:LANES]
                q = qfull.astype(BF16)
            mx = o = ls = None
            sums = []
            if icur is None:
                for c in range(NKC):
                    mx, _ = score_chunk(inext, c, q, s_next, mx)
                return mx
            mrow_b = jnp.broadcast_to(jnp.max(mx_cur, axis=-1, keepdims=True), (TM, LANES))
            EN, CN = CFG['EXP_NT'], CFG['CONV_NT']
            ocs = [qfull]
            for c in range(NKC):
                prev = ocs[c]
                pace = prev[:, EN * LANES:(EN + 1) * LANES] if (prev is not None and 'nopace' not in CFG['ABL']) else None
                o, ls, oc = pv_chunk(icur, c, s_cur, mrow_b, o, ls, pace)
                if inext is None and iconv is not None and c < NKC - 1:
                    sums += conv_paced(iconv, c, NKC - 1, oc)
                ocs.append(oc)
            last_started = ocs[-1][0:8, 0:LANES]
            NCV = CFG['NCV']
            sidx = 0

            def total(vals):
                t = None
                for v in vals:
                    t = v if t is None else t + v
                return t

            def do_scores(n, tie=None):
                nonlocal mx, sidx, sums
                for _ in range(n):
                    if inext is None or sidx >= NKC:
                        return
                    t = tie
                    if sidx == NKC - 1 and iconv is not None and CFG['CONV_FORCE'] == 's7':
                        t = total(sums) if t is None else t + total(sums)
                    mx, sfull = score_chunk(inext, sidx, _tie_bf16(q32, q, t), s_next, mx)
                    if iconv is not None and sidx < NCV:
                        sums += conv_paced(iconv, sidx, NCV, sfull)
                    last_s[0] = sfull[TM - 8:TM, (KC - LANES):KC]
                    sidx += 1

            last_s = [last_started]
            do_scores(NKC - LAG)
            do_scores(1, last_started if LAG >= 3 else None) if LAG >= 3 else None
            tie = None
            if iconv is not None and (CFG['CONV_FORCE'] == 'o' or inext is None):
                assert len(sums) == NCC * NBLK
                tie = total(sums)
            if 'noOW' in CFG['ABL'] and inext is not None:
                x1_ref[rows(icur), :] = _tie32(o * (1.0 / jnp.sum(ls, axis=-1, keepdims=True)), tie)
                do_scores(NKC)
                return mx if iconv is None else _tie32(mx, conv_stats(iconv, sums, last_started))
            x2, o_started = out_proj(icur, o, ls, tie)
            if 'noW' in CFG['ABL'] and inext is not None:
                do_scores(NKC, o_started)
                return mx if iconv is None else _tie32(mx, conv_stats(iconv, sums, o_started))
            do_scores(1, o_started) if LAG >= 2 else None
            tie_stats = None
            if iconv is not None and (CFG['STATS_FORCE'] == 'w' or inext is None):
                assert len(sums) == NCC * NBLK
                tie_stats = conv_stats(iconv, sums, last_s[0])
            elif iconv is not None and CFG['CONV_FORCE'] == 'w':
                tie_stats = total(sums)
            w_started = glu(icur, x2, tie_stats)
            do_scores(1, w_started) if LAG >= 1 else None
            if inext is not None and iconv is not None and CFG['STATS_FORCE'] == 'end':
                mx = _tie32(mx, conv_stats(iconv, sums, CFG['STATS_START'] and o_started or None) if False else conv_stats(iconv, sums, w_started if CFG['STATS_START'] else None))
            return mx

        with _Scope('s2_Bpro'):
            mr2[0] = step(0, s2.at[0], None, None, None, None)

        def phase_b(i, carry):
            cur = i % 2
            nxt = 1 - cur
            with _Scope('z_iter'):
                mr2[nxt] = step(i + 1, s2.at[nxt], i, s2.at[cur], mr2[cur], jnp.maximum(i - 2, 0))
            return carry

        with _Scope('s3_phaseB'):
            lax.fori_loop(0, N - 2, phase_b, 0)
        with _Scope('s4_Bepi'):
            cur, nxt = (N - 2) % 2, (N - 1) % 2
            mr2[nxt] = step(N - 1, s2.at[nxt], N - 2, s2.at[cur], mr2[cur], N - 4)
            step(None, None, N - 1, s2.at[nxt], mr2[nxt], N - 3)
        with _Scope('s5_conv'):
            conv(N - 2)
            conv(N - 1)

            means = st_ref[:, 0, :]
            m2s = st_ref[:, 1, :]
            mean = jnp.mean(means, axis=0, keepdims=True)
            dm = means - mean
            m2 = jnp.sum(m2s + dm * dm * float(TM), axis=0, keepdims=True)
            bn_scale = 0.5 * lax.rsqrt(m2 * (1.0 / (B * T)) + EPS)

        wcp[WP2].wait()
        wcp[W2A].wait()
        wcp[W2B].wait()

        def ocopy(i):
            b, t0 = bt(i)
            return pltpu.make_async_copy(xv.at[rows(i)], o_hbm.at[b, pl.ds(t0, TM)], osem.at[i])

        def pre_a(i, pace=None):
            u = (_pace_rows(dc_ref[rows(i), :], pace) - mean) * bn_scale
            a = _silu_half(u).astype(BF16)
            return x1_ref[rows(i), :] + _dot(a, wp2[...])

        def pre_b(x3, x3_ref, hc_ref, pace=None):
            x3_ref[...] = x3
            hc_ref[...] = _ln_scaled(_pace_rows(x3, pace), 0.5).astype(BF16)

        def ffn2(i, x3_ref, hc_ref, hooks=None):
            y = ffn(hc_ref[...], w2a, w2b, hooks=hooks)
            x1_ref[rows(i), :] = x3_ref[...] + 0.5 * y

        def post(i, pace=None):
            xv[rows(i), :] = _ln_scaled(_pace_rows(x1_ref[rows(i), :], pace), 1.0).astype(BF16)

        with _Scope('s6_Cpro'):
            pre_b(pre_a(0), x3_a, hc_a)

        def half(i, cur, nxt, do_pre, do_post):
            PA, PB, PP = CFG['C_PACE']
            box = {}
            hooks = {}

            def add(c, fn):
                if c is None:
                    fn(None)
                else:
                    prev = hooks.get(c)
                    hooks[c] = fn if prev is None else (lambda u, p=prev, f=fn: (p(u), f(u)))

            if do_pre:
                add(PA, lambda u: box.__setitem__('x3', pre_a(i + 1, u)))
                add(PB, lambda u: pre_b(box['x3'], nxt[0], nxt[1], u))
            if do_post:
                add(PP, lambda u: post(i - 1, u))
            ffn2(i, cur[0], cur[1], hooks)

        A, Bf = (x3_a, hc_a), (x3_b, hc_b)

        def pair(i, first, last):
            half(i, A, Bf, True, not first)
            half(i + 1, Bf, A, not last, True)
            if not first:
                ocopy(i - 1).start()
            ocopy(i).start()

        if CFG['OLDC']:
            def pair(i, first, last):
                pre_b(pre_a(i + 1), x3_b, hc_b)
                if not first:
                    post(i - 1)
                ffn2(i, x3_a, hc_a)
                post(i)
                if not last:
                    pre_b(pre_a(i + 2), x3_a, hc_a)
                ffn2(i + 1, x3_b, hc_b)
                if not first:
                    ocopy(i - 1).start()
                ocopy(i).start()

        def phase_c(j, carry):
            pair(2 * j, False, False)
            return carry

        with _Scope('s7_phaseC'):
            pair(0, True, False)
            lax.fori_loop(1, N // 2 - 1, phase_c, 0)
            pair(N - 2, False, True)
        with _Scope('s8_tail'):
            post(N - 1)
            ocopy(N - 1).start()
            for i in range(N):
                ocopy(i).wait()

    any_spec = pl.BlockSpec(memory_space=pl.ANY)
    scratch = [
        pltpu.VMEM((B * T, D), BF16),
        pltpu.VMEM((D, Fd), BF16), pltpu.VMEM((Fd, D), BF16),
        pltpu.VMEM((D, D), BF16), pltpu.VMEM((D, D), BF16), pltpu.VMEM((D, D), BF16), pltpu.VMEM((D, D), BF16),
        pltpu.VMEM((D, 2 * D), BF16), pltpu.VMEM((K, D), BF16), pltpu.VMEM((D, D), BF16),
        pltpu.VMEM((D, Fd), BF16), pltpu.VMEM((Fd, D), BF16),
        pltpu.VMEM((D, D), BF16), pltpu.VMEM((D, D), BF16),
        pltpu.VMEM((B * T, D), F32),
        pltpu.VMEM((B, TP, D), BF16),
        pltpu.VMEM((2, TM, TP + CFG['SPAD']), F32),
        pltpu.VMEM((B, NCC, GROWS, LANES), F32),
        pltpu.VMEM((B * T, D), F32),
        pltpu.VMEM((N, 8, D), F32),
        pltpu.VMEM((TM, D), BF16), pltpu.VMEM((TM, D), BF16),
        pltpu.VMEM((TM, D), F32), pltpu.VMEM((TM, D), F32),
        pltpu.VMEM((2, TM, LANES), F32),
        pltpu.VMEM((2, TM, D), BF16),
        pltpu.SemaphoreType.DMA((9,)),
        pltpu.SemaphoreType.DMA((2 * NFC,)),
        pltpu.SemaphoreType.DMA((N,)),
        pltpu.SemaphoreType.DMA((N,)),
    ]
    return pl.pallas_call(
        kernel,
        out_shape=jax.ShapeDtypeStruct((B, T, D), x.dtype),
        in_specs=[any_spec] * 12,
        out_specs=any_spec,
        scratch_shapes=scratch,
        compiler_params=pltpu.CompilerParams(vmem_limit_bytes=CFG['vmem_mb'] * 1024 * 1024, flags=CFG['flags']),
    )(x, w_ff1_a, w_ff1_b, w_q, w_k, w_v, w_o, w_pw1, dw, w_pw2, w_ff2_a, w_ff2_b)
```

```python
import math
import numpy as np
import jax
import jax.numpy as jnp
from jax import lax
import jax.experimental.pallas as pl
import jax.experimental.pallas.tpu as pltpu

CFG = dict(TM=400, FC=512, KC=512, RB=40, vmem_mb=120,
           flags={'XLA_TPU_EVENLY_DISTRIBUTE_CRITICAL_NODES': True},
           LAG=3, NPIECE=8, EXP_NT=0, CONV_NT=2, POLY=True, FPOLY=False, OLDC=False, SPAD=0, A_CARRY=False, A_PACE=(1, 2), C_PACE=(0, 1, 2), ABL='', NCV=6, CONV_FORCE='s7', STATS_FORCE='end', STATS_START=True, SCOPES=False,
           A_TIES=False, C_TIES=False)

F32 = jnp.float32
BF16 = jnp.bfloat16
EPS = 1e-5
LANES = 128


def _ln_scaled(x, post):
    mu = jnp.mean(x, axis=-1, keepdims=True)
    xc = x - mu
    var = jnp.mean(xc * xc, axis=-1, keepdims=True)
    inv = lax.rsqrt(var + EPS)
    if post != 1.0:
        inv = inv * post
    return xc * inv


def _dot(a, b):
    return jnp.dot(a, b, preferred_element_type=F32)


def _dot_nt(a, b):
    return lax.dot_general(a, b, (((1,), (1,)), ((), ())), preferred_element_type=F32)


def _tie32(x, on):
    if on is None:
        return x
    top = x[0:8, 0:LANES] + 0.0 * on
    row0 = jnp.concatenate([top, x[0:8, LANES:]], axis=1) if x.shape[1] > LANES else top
    return jnp.concatenate([row0, x[8:, :]], axis=0)


def _tie_bf16(x32, xb, on):
    if on is None:
        return xb
    z = 0.0 * on
    top = jnp.concatenate([x32[0:8, :] + z, x32[8:16, :] + z], axis=0).astype(BF16)
    row0 = jnp.concatenate([top, xb[0:16, LANES:]], axis=1)
    return jnp.concatenate([row0, xb[16:, :]], axis=0)


def _spread(res):
    nr = res.shape[0] // 8
    nt = res.shape[1] // LANES
    out = []
    for r in range(nr):
        j, rr = divmod(r * nt, nr)
        out.append(res[rr * 8:(rr + 1) * 8, j * LANES:(j + 1) * LANES])
    return jnp.concatenate(out, axis=0)


def _pace_rows(x, res):
    if res is None:
        return x
    left = x[:, 0:LANES] + 0.0 * _spread(res)
    return jnp.concatenate([left, x[:, LANES:]], axis=1)


def _pack_cols(v):
    return [pltpu.bitcast(v[:, c * LANES:(c + 1) * LANES], jnp.uint32) for c in range(v.shape[1] // LANES)]


def _unpack_cols(chunks):
    return jnp.concatenate([pltpu.bitcast(c, BF16) for c in chunks], axis=1)


def _silu_half(u):
    return u + u * jnp.tanh(u)


class _Scope:
    def __init__(self, name):
        self.cm = jax.named_scope(name) if CFG['SCOPES'] else None

    def __enter__(self):
        if self.cm is not None:
            self.cm.__enter__()

    def __exit__(self, *a):
        if self.cm is not None:
            self.cm.__exit__(*a)


@jax.jit
def pallas_standalone__conformer_family_conformer__speech_kernel(
    x, w_ff1_a, w_ff1_b, w_q, w_k, w_v, w_o, w_pw1, dw, w_pw2, w_ff2_a, w_ff2_b,
):
    B, T, D = x.shape
    Fd = w_ff1_a.shape[1]
    K = dw.shape[0]
    TM, FC, KC, RB = CFG['TM'], CFG['FC'], CFG['KC'], CFG['RB']
    NT = T // TM
    N = B * NT
    NFC = Fd // FC
    TP = ((T + KC - 1) // KC) * KC
    NKC = TP // KC
    PAD = K // 2
    HALO = 8
    GROWS = T + 2 * HALO
    NCC = D // LANES
    NBLK = TM // RB
    qscale = (D ** -0.5) * math.log2(math.e)

    def rows(i):
        return pl.ds(pl.multiple_of(i * TM, 16), TM)

    def bt(i):
        b = i // NT
        return b, pl.multiple_of((i - b * NT) * TM, 16)

    def kernel(x_hbm, w1a_h, w1b_h, wq_h, wk_h, wv_h, wo_h, wp1_h, dw_h, wp2_h, w2a_h, w2b_h,
               o_hbm,
               xv, w1a, w1b, wq, wk, wv, wo, wp1, dwv, wp2, w2a, w2b,
               m_ref, wvo_ref, x1_ref, h_ref, s2, g_ref, dc_ref, st_ref,
               hc_a, hc_b, x3_a, x3_b, mr2, hbuf,
               wsem, csem, xsem, osem):
        srcs = [wq_h, wk_h, wv_h, wo_h, wp1_h, dw_h, wp2_h, w2a_h, w2b_h]
        dsts = [wq, wk, wv, wo, wp1, dwv, wp2, w2a, w2b]
        wcp = [pltpu.make_async_copy(s, d, wsem.at[i]) for i, (s, d) in enumerate(zip(srcs, dsts))]
        WQ, WK, WV, WO, WP1, DW, WP2, W2A, W2B = range(9)
        acp = [pltpu.make_async_copy(w1a_h.at[:, pl.ds(c * FC, FC)], w1a.at[:, pl.ds(c * FC, FC)], csem.at[c])
               for c in range(NFC)]
        bcp = [pltpu.make_async_copy(w1b_h.at[pl.ds(c * FC, FC)], w1b.at[pl.ds(c * FC, FC)], csem.at[NFC + c])
               for c in range(NFC)]

        def xcopy(i):
            b, t0 = bt(i)
            return pltpu.make_async_copy(x_hbm.at[b, pl.ds(t0, TM)], xv.at[rows(i)], xsem.at[i])

        xcopy(0).start()
        acp[0].start()
        bcp[0].start()

        zrow = jnp.zeros((HALO, LANES), F32)
        for b in range(B):
            for cc in range(NCC):
                h_ref[b, cc, T // 2:TP // 2, :] = jnp.zeros(((TP - T) // 2, LANES), jnp.uint32)
            for cc in range(NCC):
                g_ref[b, cc, 0:HALO, :] = zrow
                g_ref[b, cc, HALO + T:GROWS, :] = zrow
        for cc in range(NCC):
            g_ref[0, cc, HALO:2 * HALO + TM, :] = jnp.zeros((TM + HALO, LANES), F32)

        def h_load(b, start, size):
            half = start // 2 if isinstance(start, int) else pl.multiple_of(start // 2, 8)
            return _unpack_cols([h_ref[b, cc, pl.ds(half, size // 2), :] for cc in range(NCC)])

        def w_load(ref):
            return _unpack_cols([ref[cc] for cc in range(NCC)])

        def w_store(ref, v):
            for cc, ch in enumerate(_pack_cols(v)):
                ref[cc] = ch

        def ffn(h_half, wa_ref, wb_ref, before_chunk=None, hooks=None):
            y = None
            for c in range(NFC):
                if before_chunk is not None:
                    before_chunk(c)
                u = _dot(h_half, wa_ref[:, c * FC:(c + 1) * FC])
                if hooks is not None and hooks.get(c) is not None:
                    hooks[c](u)
                a = _silu_half(u).astype(BF16)
                yc = _dot(a, wb_ref[c * FC:(c + 1) * FC, :])
                y = yc if y is None else y + yc
            return y

        def ln_in(i, pace=None):
            return _ln_scaled(_pace_rows(xv[rows(i), :].astype(F32), pace), 0.5).astype(BF16)

        def h1_store(i, pace=None):
            b, t0 = bt(i)
            hv = _ln_scaled(_pace_rows(x1_ref[rows(i), :], pace), 1.0).astype(BF16)
            for cc, ch in enumerate(_pack_cols(hv)):
                h_ref[b, cc, pl.ds(pl.multiple_of(t0 // 2, 8), TM // 2), :] = ch

        def a_tile(i, cur, first=False, do_post=True, do_next=True):
            P0, P1 = CFG['A_PACE']
            hooks = {}
            if do_next:
                def next_h(u):
                    hbuf[1 - cur] = ln_in(jnp.minimum(i + 1, N - 1), u)
                hooks[P0] = next_h
            if do_post:
                hooks[P1] = lambda u: h1_store(i - 1, u)

            def wait_chunk(c):
                acp[c].wait()
                bcp[c].wait()
                if c == 0:
                    acp[2].start()
                    bcp[2].start()
                    acp[3].start()
                    bcp[3].start()
                    xcopy(2).start()
                if c == 1:
                    xcopy(1).wait()
                    for k in (WQ, WK, WV, WO):
                        wcp[k].start()
                if c == 2:
                    for j in range(3, N):
                        xcopy(j).start()
                    for k in (WP1, DW, WP2, W2A, W2B):
                        wcp[k].start()

            y = ffn(hbuf[cur], w1a, w1b, wait_chunk if first else None, hooks)
            x1_ref[rows(i), :] = xv[rows(i), :].astype(F32) + 0.5 * y

        with _Scope('s0_first'):
            xcopy(0).wait()
            acp[1].start()
            bcp[1].start()
            xcopy(1).start()
            hbuf[0] = ln_in(0)
            a_tile(0, 0, first=True, do_post=False)
            xcopy(2).wait()
            a_tile(1, 1)

        def phase_a(j, carry):
            i = 2 * j
            xcopy(i + 1).wait()

            @pl.when(i + 2 < N)
            def _():
                xcopy(i + 2).wait()

            a_tile(i, 0)
            a_tile(i + 1, 1)
            return carry

        with _Scope('s1_phaseA'):
            lax.fori_loop(1, N // 2, phase_a, 0)

        with _Scope('s1b_fold'):
            for k in (WQ, WK, WV, WO):
                wcp[k].wait()
            w_store(m_ref, (_dot_nt(wq[...], wk[...]) * qscale).astype(BF16))
            w_store(wvo_ref, _dot(wv[...], wo[...]).astype(BF16))
            h1_store(N - 1)
            wcp[WP1].wait()
            wcp[DW].wait()

        def score_chunk(i, c, q, s_ref, mx):
            b = i // NT
            s = _dot_nt(q, h_load(b, c * KC, KC))
            if (c + 1) * KC > T:
                col = lax.broadcasted_iota(jnp.int32, (TM, KC), 1)
                s = jnp.where(col < T - c * KC, s, -jnp.inf)
            s_ref[:, c * KC:(c + 1) * KC] = s
            for j in range(KC // LANES):
                sj = s[:, j * LANES:(j + 1) * LANES]
                mx = sj if mx is None else jnp.maximum(mx, sj)
            return mx, s

        def pv_chunk(i, c, s_ref, mrow_b, o, ls, pace=None):
            b = i // NT
            if pace is not None:
                mrow_b = mrow_b + 0.0 * pace
            p = s_ref[:, c * KC:(c + 1) * KC] - jnp.concatenate([mrow_b] * (KC // LANES), axis=1)
            p = p if 'noexp' in CFG['ABL'] else jnp.exp2(p)
            for j in range(KC // LANES):
                pj = p[:, j * LANES:(j + 1) * LANES]
                ls = pj if ls is None else ls + pj
            oc = _dot(p.astype(BF16), h_load(b, c * KC, KC))
            return (oc if o is None else o + oc), ls, oc

        def out_proj(i, o, ls, tie=None):
            lrow = jnp.sum(ls, axis=-1, keepdims=True)
            o = _tie32(o * (1.0 / lrow), tie)
            attn = _dot(o.astype(BF16), w_load(wvo_ref))
            x2 = x1_ref[rows(i), :] + attn
            x1_ref[rows(i), :] = x2
            return x2, attn[0:8, 0:LANES]

        def glu(i, x2, tie=None):
            b, t0 = bt(i)
            h2 = _tie32(_ln_scaled(x2, 1.0), tie).astype(BF16)
            pw = _dot(h2, wp1[...])
            g = pw[:, :D] * (0.5 + 0.5 * jnp.tanh(0.5 * pw[:, D:]))
            for cc in range(NCC):
                g_ref[b, cc, pl.ds(pl.multiple_of(t0 + HALO, 8), TM), :] = g[:, cc * LANES:(cc + 1) * LANES]
            return pw[0:8, 0:LANES]

        def conv_block(i, k, pace=None, poly=None):
            b, t0 = bt(i)
            r0 = pl.multiple_of(i * TM, 16)
            cc, rb = divmod(k, NBLK)
            poly = CFG['POLY'] if poly is None else poly
            off = rb * RB
            dwf = dwv[:, cc * LANES:(cc + 1) * LANES].astype(F32)
            w = [jnp.broadcast_to(dwf[kk:kk + 1, :], (8, LANES)) for kk in range(K)]
            if pace is not None:
                z = 0.0 * pace
                w = [wk + z for wk in w] if poly else [w[0] + z] + w[1:]
            if poly:
                wt = [jnp.concatenate([wk] * (RB // 8 + 1), axis=0) for wk in w]
                ga = [g_ref[b, cc, pl.ds(pl.multiple_of(t0 + (off + 8 * a), 8), RB + 8), :] for a in range(2)]
                acc = None
                for sft in range(8):
                    zs = None
                    for a in range(2):
                        kk = 8 * a + sft - (HALO - PAD)
                        if 0 <= kk < K:
                            term = ga[a] * wt[kk]
                            zs = term if zs is None else zs + term
                    part = zs[sft:sft + RB, :]
                    acc = part if acc is None else acc + part
            else:
                wt = [jnp.concatenate([wk] * (RB // 8), axis=0) for wk in w]
                acc = None
                for kk in range(K):
                    if 'aligned' in CFG['ABL']:
                        v = g_ref[b, cc, pl.ds(pl.multiple_of(t0 + (off + 8 * kk), 8), RB), :] if False else g_ref[b, cc, pl.ds(pl.multiple_of(t0 + (off + 8 * (kk % 3)), 8), RB), :] + float(kk)
                    else:
                        v = g_ref[b, cc, pl.ds(t0 + (off + HALO - PAD + kk), RB), :]
                    term = v * wt[kk]
                    acc = term if acc is None else acc + term
            dc_ref[pl.ds(pl.multiple_of(r0 + off, 8), RB), cc * LANES:(cc + 1) * LANES] = acc
            ssum = None
            for j in range(RB // 8):
                aj = acc[j * 8:(j + 1) * 8, :]
                ssum = aj if ssum is None else ssum + aj
            return ssum

        def conv_paced(i, c, nchunks, res):
            nb = NCC * NBLK
            k0, k1 = c * nb // nchunks, (c + 1) * nb // nchunks
            out = []
            npass = res.shape[1] // LANES
            for k in range(k0, k1):
                pos = (k - k0) * npass * (TM // 8) // (k1 - k0)
                nt, r = divmod(pos, TM // 8)
                out.append(conv_block(i, k, res[r * 8:(r + 1) * 8, nt * LANES:(nt + 1) * LANES]))
            return out

        def conv_stats(i, sums, start_tie=None):
            r0 = pl.multiple_of(i * TM, 16)
            cols = []
            for cc in range(NCC):
                sc = sums[cc * NBLK]
                for rb in range(1, NBLK):
                    sc = sc + sums[cc * NBLK + rb]
                if start_tie is not None:
                    sc = sc + 0.0 * start_tie
                cols.append(jnp.sum(sc, axis=0, keepdims=True))
            mean_i = jnp.concatenate(cols, axis=1) * (1.0 / TM)
            dev = dc_ref[pl.ds(r0, TM), :] - mean_i
            m2_i = jnp.sum(dev * dev, axis=0, keepdims=True)
            st_ref[i, 0:1, :] = mean_i
            st_ref[i, 1:2, :] = m2_i
            return jnp.broadcast_to(m2_i[:, 0:LANES], (8, LANES))

        def conv(i):
            conv_stats(i, [conv_block(i, k, poly=CFG['FPOLY']) for k in range(NCC * NBLK)])

        def step(inext, s_next, icur, s_cur, mx_cur, iconv):
            LAG = CFG['LAG'] if (inext is not None and icur is not None) else 0
            q32 = q = qfull = None
            if inext is not None:
                b, t0 = bt(inext)
                qfull = _dot(h_load(b, t0, TM), w_load(m_ref))
                q32 = qfull[0:16, 0:LANES]
                q = qfull.astype(BF16)
            mx = o = ls = None
            sums = []
            if icur is None:
                for c in range(NKC):
                    mx, _ = score_chunk(inext, c, q, s_next, mx)
                return mx
            mrow_b = jnp.broadcast_to(jnp.max(mx_cur, axis=-1, keepdims=True), (TM, LANES))
            EN, CN = CFG['EXP_NT'], CFG['CONV_NT']
            ocs = [qfull]
            for c in range(NKC):
                prev = ocs[c]
                pace = prev[:, EN * LANES:(EN + 1) * LANES] if (prev is not None and 'nopace' not in CFG['ABL']) else None
                o, ls, oc = pv_chunk(icur, c, s_cur, mrow_b, o, ls, pace)
                if inext is None and iconv is not None and c < NKC - 1:
                    sums += conv_paced(iconv, c, NKC - 1, oc)
                ocs.append(oc)
            last_started = ocs[-1][0:8, 0:LANES]
            NCV = CFG['NCV']
            sidx = 0

            def total(vals):
                t = None
                for v in vals:
                    t = v if t is None else t + v
                return t

            def do_scores(n, tie=None):
                nonlocal mx, sidx, sums
                for _ in range(n):
                    if inext is None or sidx >= NKC:
                        return
                    t = tie
                    if sidx == NKC - 1 and iconv is not None and CFG['CONV_FORCE'] == 's7':
                        t = total(sums) if t is None else t + total(sums)
                    mx, sfull = score_chunk(inext, sidx, _tie_bf16(q32, q, t), s_next, mx)
                    if iconv is not None and sidx < NCV:
                        sums += conv_paced(iconv, sidx, NCV, sfull)
                    last_s[0] = sfull[TM - 8:TM, (KC - LANES):KC]
                    sidx += 1

            last_s = [last_started]
            do_scores(NKC - LAG)
            do_scores(1, last_started if LAG >= 3 else None) if LAG >= 3 else None
            tie = None
            if iconv is not None and (CFG['CONV_FORCE'] == 'o' or inext is None):
                assert len(sums) == NCC * NBLK
                tie = total(sums)
            if 'noOW' in CFG['ABL'] and inext is not None:
                x1_ref[rows(icur), :] = _tie32(o * (1.0 / jnp.sum(ls, axis=-1, keepdims=True)), tie)
                do_scores(NKC)
                return mx if iconv is None else _tie32(mx, conv_stats(iconv, sums, last_started))
            x2, o_started = out_proj(icur, o, ls, tie)
            if 'noW' in CFG['ABL'] and inext is not None:
                do_scores(NKC, o_started)
                return mx if iconv is None else _tie32(mx, conv_stats(iconv, sums, o_started))
            do_scores(1, o_started) if LAG >= 2 else None
            tie_stats = None
            if iconv is not None and (CFG['STATS_FORCE'] == 'w' or inext is None):
                assert len(sums) == NCC * NBLK
                tie_stats = conv_stats(iconv, sums, last_s[0])
            elif iconv is not None and CFG['CONV_FORCE'] == 'w':
                tie_stats = total(sums)
            w_started = glu(icur, x2, tie_stats)
            do_scores(1, w_started) if LAG >= 1 else None
            if inext is not None and iconv is not None and CFG['STATS_FORCE'] == 'end':
                mx = _tie32(mx, conv_stats(iconv, sums, CFG['STATS_START'] and o_started or None) if False else conv_stats(iconv, sums, w_started if CFG['STATS_START'] else None))
            return mx

        with _Scope('s2_Bpro'):
            mr2[0] = step(0, s2.at[0], None, None, None, None)

        def phase_b(i, carry):
            cur = i % 2
            nxt = 1 - cur
            with _Scope('z_iter'):
                mr2[nxt] = step(i + 1, s2.at[nxt], i, s2.at[cur], mr2[cur], jnp.maximum(i - 2, 0))
            return carry

        with _Scope('s3_phaseB'):
            lax.fori_loop(0, N - 1, phase_b, 0)
        with _Scope('s4_Bepi'):
            step(None, None, N - 1, s2.at[(N - 1) % 2], mr2[(N - 1) % 2], N - 3)
        with _Scope('s5_conv'):
            conv(N - 2)
            conv(N - 1)

            means = st_ref[:, 0, :]
            m2s = st_ref[:, 1, :]
            mean = jnp.mean(means, axis=0, keepdims=True)
            dm = means - mean
            m2 = jnp.sum(m2s + dm * dm * float(TM), axis=0, keepdims=True)
            bn_scale = 0.5 * lax.rsqrt(m2 * (1.0 / (B * T)) + EPS)

        wcp[WP2].wait()
        wcp[W2A].wait()
        wcp[W2B].wait()

        def ocopy(i):
            b, t0 = bt(i)
            return pltpu.make_async_copy(xv.at[rows(i)], o_hbm.at[b, pl.ds(t0, TM)], osem.at[i])

        def pre_a(i, pace=None):
            u = (_pace_rows(dc_ref[rows(i), :], pace) - mean) * bn_scale
            a = _silu_half(u).astype(BF16)
            return x1_ref[rows(i), :] + _dot(a, wp2[...])

        def pre_b(x3, x3_ref, hc_ref, pace=None):
            x3_ref[...] = x3
            hc_ref[...] = _ln_scaled(_pace_rows(x3, pace), 0.5).astype(BF16)

        def ffn2(i, x3_ref, hc_ref, hooks=None):
            y = ffn(hc_ref[...], w2a, w2b, hooks=hooks)
            x1_ref[rows(i), :] = x3_ref[...] + 0.5 * y

        def post(i, pace=None):
            xv[rows(i), :] = _ln_scaled(_pace_rows(x1_ref[rows(i), :], pace), 1.0).astype(BF16)

        with _Scope('s6_Cpro'):
            pre_b(pre_a(0), x3_a, hc_a)

        def half(i, cur, nxt, do_pre, do_post):
            PA, PB, PP = CFG['C_PACE']
            box = {}
            hooks = {}

            def add(c, fn):
                if c is None:
                    fn(None)
                else:
                    prev = hooks.get(c)
                    hooks[c] = fn if prev is None else (lambda u, p=prev, f=fn: (p(u), f(u)))

            if do_pre:
                add(PA, lambda u: box.__setitem__('x3', pre_a(i + 1, u)))
                add(PB, lambda u: pre_b(box['x3'], nxt[0], nxt[1], u))
            if do_post:
                add(PP, lambda u: post(i - 1, u))
            ffn2(i, cur[0], cur[1], hooks)

        A, Bf = (x3_a, hc_a), (x3_b, hc_b)

        def pair(i, first, last):
            half(i, A, Bf, True, not first)
            half(i + 1, Bf, A, not last, True)
            if not first:
                ocopy(i - 1).start()
            ocopy(i).start()

        if CFG['OLDC']:
            def pair(i, first, last):
                pre_b(pre_a(i + 1), x3_b, hc_b)
                if not first:
                    post(i - 1)
                ffn2(i, x3_a, hc_a)
                post(i)
                if not last:
                    pre_b(pre_a(i + 2), x3_a, hc_a)
                ffn2(i + 1, x3_b, hc_b)
                if not first:
                    ocopy(i - 1).start()
                ocopy(i).start()

        def phase_c(j, carry):
            pair(2 * j, False, False)
            return carry

        with _Scope('s7_phaseC'):
            pair(0, True, False)
            lax.fori_loop(1, N // 2 - 1, phase_c, 0)
            pair(N - 2, False, True)
        with _Scope('s8_tail'):
            post(N - 1)
            ocopy(N - 1).start()
            for i in range(N):
                ocopy(i).wait()

    any_spec = pl.BlockSpec(memory_space=pl.ANY)
    scratch = [
        pltpu.VMEM((B * T, D), BF16),
        pltpu.VMEM((D, Fd), BF16), pltpu.VMEM((Fd, D), BF16),
        pltpu.VMEM((D, D), BF16), pltpu.VMEM((D, D), BF16), pltpu.VMEM((D, D), BF16), pltpu.VMEM((D, D), BF16),
        pltpu.VMEM((D, 2 * D), BF16), pltpu.VMEM((K, D), BF16), pltpu.VMEM((D, D), BF16),
        pltpu.VMEM((D, Fd), BF16), pltpu.VMEM((Fd, D), BF16),
        pltpu.VMEM((NCC, D // 2, LANES), jnp.uint32), pltpu.VMEM((NCC, D // 2, LANES), jnp.uint32),
        pltpu.VMEM((B * T, D), F32),
        pltpu.VMEM((B, NCC, TP // 2, LANES), jnp.uint32),
        pltpu.VMEM((2, TM, TP + CFG['SPAD']), F32),
        pltpu.VMEM((B, NCC, GROWS, LANES), F32),
        pltpu.VMEM((B * T, D), F32),
        pltpu.VMEM((N, 8, D), F32),
        pltpu.VMEM((TM, D), BF16), pltpu.VMEM((TM, D), BF16),
        pltpu.VMEM((TM, D), F32), pltpu.VMEM((TM, D), F32),
        pltpu.VMEM((2, TM, LANES), F32),
        pltpu.VMEM((2, TM, D), BF16),
        pltpu.SemaphoreType.DMA((9,)),
        pltpu.SemaphoreType.DMA((2 * NFC,)),
        pltpu.SemaphoreType.DMA((N,)),
        pltpu.SemaphoreType.DMA((N,)),
    ]
    return pl.pallas_call(
        kernel,
        out_shape=jax.ShapeDtypeStruct((B, T, D), x.dtype),
        in_specs=[any_spec] * 12,
        out_specs=any_spec,
        scratch_shapes=scratch,
        compiler_params=pltpu.CompilerParams(vmem_limit_bytes=CFG['vmem_mb'] * 1024 * 1024, flags=CFG['flags']),
    )(x, w_ff1_a, w_ff1_b, w_q, w_k, w_v, w_o, w_pw1, dw, w_pw2, w_ff2_a, w_ff2_b)
```

```python
import math
import numpy as np
import jax
import jax.numpy as jnp
from jax import lax
import jax.experimental.pallas as pl
import jax.experimental.pallas.tpu as pltpu

CFG = dict(TM=400, FC=512, KC=512, RB=16, vmem_mb=120,
           flags={'XLA_TPU_EVENLY_DISTRIBUTE_CRITICAL_NODES': True},
           LAG=3, NPIECE=8, EXP_NT=1, BX2=False, LATE_MAX=False, XCONV=True, STAT_G=10, STAT_W=1024, START=1, A0FIRST=True, NOC=False, CONV_NT=2, POLY=True, FPOLY=False, OLDC=False, SPAD=0, A_CARRY=False, A_PACE=(1, 2), C_PACE=(0, 1, 2), ABL='', NCV=5, CONV_FORCE='s7', STATS_FORCE='end', STATS_START=True, SCOPES=False,
           A_TIES=False, C_TIES=False)

F32 = jnp.float32
BF16 = jnp.bfloat16
EPS = 1e-5
LANES = 128


def _ln_scaled(x, post):
    mu = jnp.mean(x, axis=-1, keepdims=True)
    xc = x - mu
    var = jnp.mean(xc * xc, axis=-1, keepdims=True)
    inv = lax.rsqrt(var + EPS)
    if post != 1.0:
        inv = inv * post
    return xc * inv


def _dot(a, b):
    return jnp.dot(a, b, preferred_element_type=F32)


def _dot_nt(a, b):
    return lax.dot_general(a, b, (((1,), (1,)), ((), ())), preferred_element_type=F32)


def _tie32(x, on):
    if on is None:
        return x
    top = x[0:8, 0:LANES] + 0.0 * on
    row0 = jnp.concatenate([top, x[0:8, LANES:]], axis=1) if x.shape[1] > LANES else top
    return jnp.concatenate([row0, x[8:, :]], axis=0)


def _tie_bf16(x32, xb, on):
    if on is None:
        return xb
    z = 0.0 * on
    top = jnp.concatenate([x32[0:8, :] + z, x32[8:16, :] + z], axis=0).astype(BF16)
    row0 = jnp.concatenate([top, xb[0:16, LANES:]], axis=1)
    return jnp.concatenate([row0, xb[16:, :]], axis=0)


def _spread(res):
    nr = res.shape[0] // 8
    nt = res.shape[1] // LANES
    out = []
    for r in range(nr):
        j, rr = divmod(r * nt, nr)
        out.append(res[rr * 8:(rr + 1) * 8, j * LANES:(j + 1) * LANES])
    return jnp.concatenate(out, axis=0)


def _pace_rows(x, res):
    if res is None:
        return x
    left = x[:, 0:LANES] + 0.0 * _spread(res)
    return jnp.concatenate([left, x[:, LANES:]], axis=1)


def _pack_cols(v):
    return [pltpu.bitcast(v[:, c * LANES:(c + 1) * LANES], jnp.uint32) for c in range(v.shape[1] // LANES)]


def _unpack_cols(chunks):
    return jnp.concatenate([pltpu.bitcast(c, BF16) for c in chunks], axis=1)


def _silu_half(u):
    return u + u * jnp.tanh(u)


class _Scope:
    def __init__(self, name):
        self.cm = jax.named_scope(name) if CFG['SCOPES'] else None

    def __enter__(self):
        if self.cm is not None:
            self.cm.__enter__()

    def __exit__(self, *a):
        if self.cm is not None:
            self.cm.__exit__(*a)


@jax.jit
def pallas_standalone__conformer_family_conformer__speech_kernel(
    x, w_ff1_a, w_ff1_b, w_q, w_k, w_v, w_o, w_pw1, dw, w_pw2, w_ff2_a, w_ff2_b,
):
    B, T, D = x.shape
    Fd = w_ff1_a.shape[1]
    K = dw.shape[0]
    TM, FC, KC, RB = CFG['TM'], CFG['FC'], CFG['KC'], CFG['RB']
    NT = T // TM
    N = B * NT
    NFC = Fd // FC
    TP = ((T + KC - 1) // KC) * KC
    NKC = TP // KC
    PAD = K // 2
    HALO = 8
    GROWS = T + 2 * HALO
    NCC = D // LANES
    NBLK = TM // RB
    qscale = (D ** -0.5) * math.log2(math.e)

    def rows(i):
        return pl.ds(pl.multiple_of(i * TM, 16), TM)

    def bt(i):
        b = i // NT
        return b, pl.multiple_of((i - b * NT) * TM, 16)

    def kernel(x_hbm, w1a_h, w1b_h, wq_h, wk_h, wv_h, wo_h, wp1_h, dw_h, wp2_h, w2a_h, w2b_h,
               o_hbm,
               xv, w1a, w1b, wq, wk, wv, wo, wp1, dwv, wp2, w2a, w2b,
               m_ref, wvo_ref, x1_ref, h_ref, s2, g_ref, dc_ref, st_ref,
               hc_a, hc_b, x3_a, x3_b, mr2, hbuf,
               wsem, csem, xsem, osem):
        srcs = [wq_h, wk_h, wv_h, wo_h, wp1_h, dw_h, wp2_h, w2a_h, w2b_h]
        dsts = [wq, wk, wv, wo, wp1, dwv, wp2, w2a, w2b]
        wcp = [pltpu.make_async_copy(s, d, wsem.at[i]) for i, (s, d) in enumerate(zip(srcs, dsts))]
        WQ, WK, WV, WO, WP1, DW, WP2, W2A, W2B = range(9)
        acp = [pltpu.make_async_copy(w1a_h.at[:, pl.ds(c * FC, FC)], w1a.at[:, pl.ds(c * FC, FC)], csem.at[c])
               for c in range(NFC)]
        bcp = [pltpu.make_async_copy(w1b_h.at[pl.ds(c * FC, FC)], w1b.at[pl.ds(c * FC, FC)], csem.at[NFC + c])
               for c in range(NFC)]

        def xcopy(i):
            b, t0 = bt(i)
            return pltpu.make_async_copy(x_hbm.at[b, pl.ds(t0, TM)], xv.at[rows(i)], xsem.at[i])

        xcopy(0).start()
        acp[0].start()
        bcp[0].start()

        zrow = jnp.zeros((HALO, LANES), F32)
        for b in range(B):
            for cc in range(NCC):
                h_ref[b, cc, T // 2:TP // 2, :] = jnp.zeros(((TP - T) // 2, LANES), jnp.uint32)
            for cc in range(NCC):
                g_ref[b, cc, 0:HALO, :] = zrow
                g_ref[b, cc, HALO + T:GROWS, :] = zrow
        for cc in range(NCC):
            g_ref[0, cc, HALO:2 * HALO + TM, :] = jnp.zeros((TM + HALO, LANES), F32)

        def h_load(b, start, size):
            half = start // 2 if isinstance(start, int) else pl.multiple_of(start // 2, 8)
            return _unpack_cols([h_ref[b, cc, pl.ds(half, size // 2), :] for cc in range(NCC)])

        def w_load(ref):
            return _unpack_cols([ref[cc] for cc in range(NCC)])

        def w_store(ref, v):
            for cc, ch in enumerate(_pack_cols(v)):
                ref[cc] = ch

        def ffn(h_half, wa_ref, wb_ref, before_chunk=None, hooks=None, before_down=None):
            y = None
            for c in range(NFC):
                if before_chunk is not None:
                    before_chunk(c)
                u = _dot(h_half, wa_ref[:, c * FC:(c + 1) * FC])
                if hooks is not None and hooks.get(c) is not None:
                    hooks[c](u)
                a = _silu_half(u).astype(BF16)
                if before_down is not None:
                    before_down(c)
                yc = _dot(a, wb_ref[c * FC:(c + 1) * FC, :])
                y = yc if y is None else y + yc
            return y

        def ln_in(i, pace=None):
            return _ln_scaled(_pace_rows(xv[rows(i), :].astype(F32), pace), 0.5).astype(BF16)

        def h1_store(i, pace=None):
            b, t0 = bt(i)
            hv = _ln_scaled(_pace_rows(x1_ref[rows(i), :], pace), 1.0).astype(BF16)
            for cc, ch in enumerate(_pack_cols(hv)):
                h_ref[b, cc, pl.ds(pl.multiple_of(t0 // 2, 8), TM // 2), :] = ch

        def a_tile(i, cur, first=False, do_post=True, do_next=True):
            P0, P1 = CFG['A_PACE']
            hooks = {}
            if do_next:
                def next_h(u):
                    hbuf[1 - cur] = ln_in(jnp.minimum(i + 1, N - 1), u)
                hooks[P0] = next_h
            if do_post:
                hooks[P1] = lambda u: h1_store(i - 1, u)

            def wait_chunk(c):
                acp[c].wait()
                if c >= 2:
                    bcp[c].wait()
                if c == 0:
                    acp[2].start()
                    bcp[2].start()
                    acp[3].start()
                    bcp[3].start()
                    xcopy(2).start()
                if c == 1:
                    for k in (WQ, WK, WV, WO):
                        wcp[k].start()
                if c == 2:
                    xcopy(1).wait()
                    for j in range(3, N):
                        xcopy(j).start()
                    for k in (WP1, DW, WP2, W2A, W2B):
                        wcp[k].start()

            if first and do_next:
                hooks = {2: next_h}

            y = ffn(hbuf[cur], w1a, w1b, wait_chunk if first else None, hooks,
                    (lambda c: bcp[c].wait() if c < 2 else None) if first else None)
            x1_ref[rows(i), :] = xv[rows(i), :].astype(F32) + 0.5 * y

        with _Scope('s0_first'):
            xcopy(0).wait()
            acp[1].start()
            bcp[1].start()
            xcopy(1).start()
            hbuf[0] = ln_in(0)
            a_tile(0, 0, first=True, do_post=False)
            xcopy(2).wait()
            a_tile(1, 1)

        def phase_a(j, carry):
            i = 2 * j
            xcopy(i + 1).wait()

            @pl.when(i + 2 < N)
            def _():
                xcopy(i + 2).wait()

            a_tile(i, 0)
            a_tile(i + 1, 1)
            return carry

        with _Scope('s1_phaseA'):
            lax.fori_loop(1, N // 2, phase_a, 0)

        with _Scope('s1b_fold'):
            for k in (WQ, WK, WV, WO):
                wcp[k].wait()
            w_store(m_ref, (_dot_nt(wq[...], wk[...]) * qscale).astype(BF16))
            w_store(wvo_ref, _dot(wv[...], wo[...]).astype(BF16))
            h1_store(N - 1)
            wcp[WP1].wait()
            wcp[DW].wait()

        def score_chunk(i, c, q, s_ref, mx):
            b = i // NT
            s = _dot_nt(q, h_load(b, c * KC, KC))
            if (c + 1) * KC > T:
                col = lax.broadcasted_iota(jnp.int32, (TM, KC), 1)
                s = jnp.where(col < T - c * KC, s, -jnp.inf)
            s_ref[:, c * KC:(c + 1) * KC] = s
            if not CFG['LATE_MAX']:
                for j in range(KC // LANES):
                    sj = s[:, j * LANES:(j + 1) * LANES]
                    mx = sj if mx is None else jnp.maximum(mx, sj)
            return mx, s

        def pv_chunk(i, c, s_ref, mrow_b, o, ls, pace=None):
            b = i // NT
            if pace is not None:
                mrow_b = mrow_b + 0.0 * pace
            p = s_ref[:, c * KC:(c + 1) * KC] - jnp.concatenate([mrow_b] * (KC // LANES), axis=1)
            p = p if 'noexp' in CFG['ABL'] else jnp.exp2(p)
            for j in range(KC // LANES):
                pj = p[:, j * LANES:(j + 1) * LANES]
                ls = pj if ls is None else ls + pj
            oc = _dot(p.astype(BF16), h_load(b, c * KC, KC))
            return (oc if o is None else o + oc), ls, oc

        def out_proj(i, o, ls, tie=None):
            lrow = jnp.sum(ls, axis=-1, keepdims=True)
            o = _tie32(o * (1.0 / lrow), tie)
            attn = _dot(o.astype(BF16), w_load(wvo_ref))
            x2 = x1_ref[rows(i), :] + attn
            x1_ref[rows(i), :] = x2
            return x2, attn

        def glu(i, x2, tie=None):
            b, t0 = bt(i)
            h2 = _tie32(_ln_scaled(x2, 1.0), tie).astype(BF16)
            pw = _dot(h2, wp1[...])
            g = pw[:, :D] * (0.5 + 0.5 * jnp.tanh(0.5 * pw[:, D:]))
            for cc in range(NCC):
                g_ref[b, cc, pl.ds(pl.multiple_of(t0 + HALO, 8), TM), :] = g[:, cc * LANES:(cc + 1) * LANES]
            return pw

        def conv_block(i, k, pace=None, poly=None):
            b, t0 = bt(i)
            r0 = pl.multiple_of(i * TM, 16)
            cc, rb = divmod(k, NBLK)
            poly = CFG['POLY'] if poly is None else poly
            off = rb * RB
            dwf = dwv[:, cc * LANES:(cc + 1) * LANES].astype(F32)
            w = [jnp.broadcast_to(dwf[kk:kk + 1, :], (8, LANES)) for kk in range(K)]
            if pace is not None:
                z = 0.0 * pace
                w = [wk + z for wk in w] if poly else [w[0] + z] + w[1:]
            if poly:
                wt = [jnp.concatenate([wk] * (RB // 8 + 1), axis=0) for wk in w]
                ga = [g_ref[b, cc, pl.ds(pl.multiple_of(t0 + (off + 8 * a), 8), RB + 8), :] for a in range(2)]
                acc = None
                for sft in range(8):
                    zs = None
                    for a in range(2):
                        kk = 8 * a + sft - (HALO - PAD)
                        if 0 <= kk < K:
                            term = ga[a] * wt[kk]
                            zs = term if zs is None else zs + term
                    part = zs[sft:sft + RB, :]
                    acc = part if acc is None else acc + part
            else:
                wt = [jnp.concatenate([wk] * (RB // 8), axis=0) for wk in w]
                acc = None
                for kk in range(K):
                    if 'aligned' in CFG['ABL']:
                        v = g_ref[b, cc, pl.ds(pl.multiple_of(t0 + (off + 8 * kk), 8), RB), :] if False else g_ref[b, cc, pl.ds(pl.multiple_of(t0 + (off + 8 * (kk % 3)), 8), RB), :] + float(kk)
                    else:
                        v = g_ref[b, cc, pl.ds(t0 + (off + HALO - PAD + kk), RB), :]
                    term = v * wt[kk]
                    acc = term if acc is None else acc + term
            dc_ref[pl.ds(pl.multiple_of(r0 + off, 8), RB), cc * LANES:(cc + 1) * LANES] = acc
            ssum = None
            for j in range(RB // 8):
                aj = acc[j * 8:(j + 1) * 8, :]
                ssum = aj if ssum is None else ssum + aj
            return ssum

        def conv_jobs(jobs, res):
            out = []
            npass = res.shape[1] // LANES
            for n, (ti, k) in enumerate(jobs):
                pos = n * npass * (TM // 8) // len(jobs)
                nt, r = divmod(pos, TM // 8)
                out.append(conv_block(ti, k, res[r * 8:(r + 1) * 8, nt * LANES:(nt + 1) * LANES]))
            return out

        def conv_paced(i, c, nchunks, res):
            nb = NCC * NBLK
            return conv_jobs([(i, k) for k in range(c * nb // nchunks, (c + 1) * nb // nchunks)], res)

        def conv_stats(i, sums, pace=None):
            r0 = pl.multiple_of(i * TM, 16)
            means, m2s = [], []
            NG = CFG['STAT_G']
            GR = TM // NG
            for cc in range(NCC):
                sc = sums[cc * NBLK]
                for rb in range(1, NBLK):
                    sc = sc + sums[cc * NBLK + rb]
                mean_c = jnp.sum(sc, axis=0, keepdims=True) * (1.0 / TM)
                means.append(mean_c)
                mean_b = jnp.broadcast_to(mean_c, (8, LANES))
                acc = None
                for gidx in range(NG):
                    mb = mean_b
                    if pace is not None:
                        npass = pace.shape[1] // LANES
                        pos = (cc * NG + gidx) * npass * (TM // 8) // (NCC * NG)
                        nt, r = divmod(pos, TM // 8)
                        mb = mb + 0.0 * pace[r * 8:(r + 1) * 8, nt * LANES:(nt + 1) * LANES]
                    blk = dc_ref[pl.ds(pl.multiple_of(r0 + gidx * GR, 8), GR), cc * LANES:(cc + 1) * LANES]
                    for j in range(GR // 8):
                        d = blk[j * 8:(j + 1) * 8, :] - mb
                        acc = d * d if acc is None else acc + d * d
                m2s.append(jnp.sum(acc, axis=0, keepdims=True))
            st_ref[i, 0:1, :] = jnp.concatenate(means, axis=1)
            st_ref[i, 1:2, :] = jnp.concatenate(m2s, axis=1)
            return jnp.broadcast_to(m2s[-1], (8, LANES))

        def conv(i):
            conv_stats(i, [conv_block(i, k, poly=CFG['FPOLY']) for k in range(NCC * NBLK)])

        def step(inext, s_next, icur, s_cur, mx_cur, iconv, xconv=None):
            LAG = CFG['LAG'] if (inext is not None and icur is not None) else 0
            q32 = q = qfull = None
            if inext is not None:
                b, t0 = bt(inext)
                qfull = _dot(h_load(b, t0, TM), w_load(m_ref))
                q32 = qfull[0:16, 0:LANES]
                q = qfull.astype(BF16)
            mx = o = ls = None
            sums = []
            xs = {}
            if icur is None:
                for c in range(NKC):
                    mx, _ = score_chunk(inext, c, q, s_next, mx)
                return mx
            if CFG['LATE_MAX']:
                mx_cur = None
                for c in range(NKC):
                    sc = s_cur[:, c * KC:(c + 1) * KC]
                    mc = jnp.maximum(jnp.maximum(sc[:, 0:LANES], sc[:, LANES:2 * LANES]),
                                     jnp.maximum(sc[:, 2 * LANES:3 * LANES], sc[:, 3 * LANES:4 * LANES]))
                    mx_cur = mc if mx_cur is None else jnp.maximum(mx_cur, mc)
            mrow_b = jnp.broadcast_to(jnp.max(mx_cur, axis=-1, keepdims=True), (TM, LANES))
            EN, CN = CFG['EXP_NT'], CFG['CONV_NT']
            ocs = [qfull]
            for c in range(NKC):
                prev = ocs[c]
                pace = prev[:, EN * LANES:(EN + 1) * LANES] if (prev is not None and 'nopace' not in CFG['ABL']) else None
                o, ls, oc = pv_chunk(icur, c, s_cur, mrow_b, o, ls, pace)
                if inext is None and iconv is not None and c < NKC - 1:
                    nb = NCC * NBLK
                    jobs = [(iconv, k) for k in range(c * nb // (NKC - 1), (c + 1) * nb // (NKC - 1))]
                    nown = len(jobs)
                    if xconv is not None:
                        xj = [(xconv, k) for k in range(nb) if (k + 1) % NBLK != 0]
                        jobs = jobs + xj[c * len(xj) // (NKC - 1):(c + 1) * len(xj) // (NKC - 1)]
                        order = sorted(range(len(jobs)), key=lambda n: (n / max(nown, 1)) if n < nown else ((n - nown + 0.5) / max(len(jobs) - nown, 1)))
                    else:
                        order = list(range(len(jobs)))
                    res = conv_jobs([jobs[n] for n in order], oc)
                    vals = [None] * len(jobs)
                    for n, v in zip(order, res):
                        vals[n] = v
                    sums += vals[:nown]
                    for (_, k), v in zip(jobs[nown:], vals[nown:]):
                        xs[k] = v
                ocs.append(oc)
            last_started = ocs[-1][0:8, 0:LANES]
            NCV = CFG['NCV']
            sidx = 0

            def total(vals):
                t = None
                for v in vals:
                    t = v if t is None else t + v
                return t

            def do_scores(n, tie=None):
                nonlocal mx, sidx, sums
                for _ in range(n):
                    if inext is None or sidx >= NKC:
                        return
                    t = tie
                    if sidx == NKC - 1 and iconv is not None and CFG['CONV_FORCE'] == 's7':
                        t = total(sums) if t is None else t + total(sums)
                    mx, sfull = score_chunk(inext, sidx, _tie_bf16(q32, q, t), s_next, mx)
                    if iconv is not None and sidx < NCV:
                        sums += conv_paced(iconv, sidx, NCV, sfull)
                    last_s[0] = sfull[TM - 8:TM, (KC - LANES):KC]
                    sidx += 1

            last_s = [last_started]
            do_scores(NKC - LAG)
            do_scores(1, last_started if LAG >= 3 else None) if LAG >= 3 else None
            tie = None
            if iconv is not None and (CFG['CONV_FORCE'] == 'o' or inext is None):
                assert len(sums) == NCC * NBLK
                tie = total(sums)
            if 'noOW' in CFG['ABL'] and inext is not None:
                x1_ref[rows(icur), :] = _tie32(o * (1.0 / jnp.sum(ls, axis=-1, keepdims=True)), tie)
                do_scores(NKC)
                return mx if iconv is None else _tie32(mx, conv_stats(iconv, sums, ocs[-1]))
            x2, attn = out_proj(icur, o, ls, tie)
            o_started = attn[0:8, 0:LANES]
            if 'noW' in CFG['ABL'] and inext is not None:
                do_scores(NKC, o_started)
                return mx if iconv is None else _tie32(mx, conv_stats(iconv, sums, attn))
            do_scores(1, o_started) if LAG >= 2 else None
            tie_stats = None
            if iconv is not None and (CFG['STATS_FORCE'] == 'w' or inext is None):
                assert len(sums) == NCC * NBLK
                tie_stats = conv_stats(iconv, sums, ocs[-1])
            elif iconv is not None and CFG['CONV_FORCE'] == 'w':
                tie_stats = total(sums)
            pw = glu(icur, x2, tie_stats)
            w_started = pw[0:8, 0:LANES]
            if xconv is not None:
                return xs
            do_scores(1, w_started) if LAG >= 1 else None
            if inext is not None and iconv is not None and CFG['STATS_FORCE'] == 'end' and CFG['LATE_MAX']:
                conv_stats(iconv, sums, pw[:, :CFG['STAT_W']] if CFG['STATS_START'] else None)
            elif inext is not None and iconv is not None and CFG['STATS_FORCE'] == 'end':
                mx = _tie32(mx, conv_stats(iconv, sums, pw[:, :CFG['STAT_W']] if CFG['STATS_START'] else None))
            return mx

        with _Scope('s2_Bpro'):
            m0 = step(0, s2.at[0], None, None, None, None)
            if not CFG['LATE_MAX']:
                mr2[0] = m0

        def phase_b(i, carry):
            cur = i % 2
            nxt = 1 - cur
            if CFG['LATE_MAX']:
                step(i + 1, s2.at[nxt], i, s2.at[cur], None, jnp.maximum(i - 2, 0))
            else:
                mr2[nxt] = step(i + 1, s2.at[nxt], i, s2.at[cur], mr2[cur], jnp.maximum(i - 2, 0))
            return carry

        def phase_b2(j, carry):
            i = 2 * j
            mr2[1] = step(i + 1, s2.at[1], i, s2.at[0], mr2[0], jnp.maximum(i - 2, 0))
            mr2[0] = step(i + 2, s2.at[0], i + 1, s2.at[1], mr2[1], jnp.maximum(i - 1, 0))
            return carry

        with _Scope('s3_phaseB'):
            if CFG['BX2']:
                lax.fori_loop(0, (N - 1) // 2, phase_b2, 0)
                phase_b(N - 2, 0)
            else:
                lax.fori_loop(0, N - 1, phase_b, 0)
        m_last = None if CFG['LATE_MAX'] else mr2[(N - 1) % 2]
        if CFG['XCONV']:
            with _Scope('s4_Bepi'):
                xs = step(None, None, N - 1, s2.at[(N - 1) % 2], m_last, N - 3, xconv=N - 2)
            with _Scope('s5_conv'):
                for k in range(NCC * NBLK):
                    if k not in xs:
                        xs[k] = conv_block(N - 2, k, poly=CFG['FPOLY'])
                conv(N - 1)
                conv_stats(N - 2, [xs[k] for k in range(NCC * NBLK)])
        else:
            with _Scope('s4_Bepi'):
                step(None, None, N - 1, s2.at[(N - 1) % 2], m_last, N - 3)
            with _Scope('s5_conv'):
                conv(N - 2)
                conv(N - 1)
        if True:
            means = st_ref[:, 0, :]
            m2s = st_ref[:, 1, :]
            mean = jnp.mean(means, axis=0, keepdims=True)
            dm = means - mean
            m2 = jnp.sum(m2s + dm * dm * float(TM), axis=0, keepdims=True)
            bn_scale = 0.5 * lax.rsqrt(m2 * (1.0 / (B * T)) + EPS)

        wcp[WP2].wait()
        wcp[W2A].wait()
        wcp[W2B].wait()

        def ocopy(i):
            b, t0 = bt(i)
            return pltpu.make_async_copy(xv.at[rows(i)], o_hbm.at[b, pl.ds(t0, TM)], osem.at[i])

        def pre_a(i, pace=None):
            u = (_pace_rows(dc_ref[rows(i), :], pace) - mean) * bn_scale
            a = _silu_half(u).astype(BF16)
            return x1_ref[rows(i), :] + _dot(a, wp2[...])

        def pre_b(x3, x3_ref, hc_ref, pace=None):
            x3_ref[...] = x3
            hc_ref[...] = _ln_scaled(_pace_rows(x3, pace), 0.5).astype(BF16)

        def ffn2(i, x3_ref, hc_ref, hooks=None):
            y = ffn(hc_ref[...], w2a, w2b, hooks=hooks)
            x1_ref[rows(i), :] = x3_ref[...] + 0.5 * y

        def post(i, pace=None):
            xv[rows(i), :] = _ln_scaled(_pace_rows(x1_ref[rows(i), :], pace), 1.0).astype(BF16)

        with _Scope('s6_Cpro'):
            pre_b(pre_a(0), x3_a, hc_a)

        def half(i, cur, nxt, do_pre, do_post):
            PA, PB, PP = CFG['C_PACE']
            box = {}
            hooks = {}

            def add(c, fn):
                if c is None:
                    fn(None)
                else:
                    prev = hooks.get(c)
                    hooks[c] = fn if prev is None else (lambda u, p=prev, f=fn: (p(u), f(u)))

            if do_pre:
                add(PA, lambda u: box.__setitem__('x3', pre_a(i + 1, u)))
                add(PB, lambda u: pre_b(box['x3'], nxt[0], nxt[1], u))
            if do_post:
                add(PP, lambda u: post(i - 1, u))
            ffn2(i, cur[0], cur[1], hooks)

        A, Bf = (x3_a, hc_a), (x3_b, hc_b)

        def pair(i, first, last):
            half(i, A, Bf, True, not first)
            half(i + 1, Bf, A, not last, True)
            if not first:
                ocopy(i - 1).start()
            ocopy(i).start()

        if CFG['OLDC']:
            def pair(i, first, last):
                pre_b(pre_a(i + 1), x3_b, hc_b)
                if not first:
                    post(i - 1)
                ffn2(i, x3_a, hc_a)
                post(i)
                if not last:
                    pre_b(pre_a(i + 2), x3_a, hc_a)
                ffn2(i + 1, x3_b, hc_b)
                if not first:
                    ocopy(i - 1).start()
                ocopy(i).start()

        def phase_c(j, carry):
            pair(2 * j, False, False)
            return carry

        with _Scope('s7_phaseC'):
            if not CFG['NOC']:
                pair(0, True, False)
                lax.fori_loop(1, N // 2 - 1, phase_c, 0)
                pair(N - 2, False, True)
            else:
                for i in range(N - 1):
                    ocopy(i).start()
        with _Scope('s8_tail'):
            post(N - 1)
            ocopy(N - 1).start()
            for i in range(N):
                ocopy(i).wait()

    any_spec = pl.BlockSpec(memory_space=pl.ANY)
    scratch = [
        pltpu.VMEM((B * T, D), BF16),
        pltpu.VMEM((D, Fd), BF16), pltpu.VMEM((Fd, D), BF16),
        pltpu.VMEM((D, D), BF16), pltpu.VMEM((D, D), BF16), pltpu.VMEM((D, D), BF16), pltpu.VMEM((D, D), BF16),
        pltpu.VMEM((D, 2 * D), BF16), pltpu.VMEM((K, D), BF16), pltpu.VMEM((D, D), BF16),
        pltpu.VMEM((D, Fd), BF16), pltpu.VMEM((Fd, D), BF16),
        pltpu.VMEM((NCC, D // 2, LANES), jnp.uint32), pltpu.VMEM((NCC, D // 2, LANES), jnp.uint32),
        pltpu.VMEM((B * T, D), F32),
        pltpu.VMEM((B, NCC, TP // 2, LANES), jnp.uint32),
        pltpu.VMEM((2, TM, TP + CFG['SPAD']), F32),
        pltpu.VMEM((B, NCC, GROWS, LANES), F32),
        pltpu.VMEM((B * T, D), F32),
        pltpu.VMEM((N, 8, D), F32),
        pltpu.VMEM((TM, D), BF16), pltpu.VMEM((TM, D), BF16),
        pltpu.VMEM((TM, D), F32), pltpu.VMEM((TM, D), F32),
        pltpu.VMEM((2, TM, LANES), F32),
        pltpu.VMEM((2, TM, D), BF16),
        pltpu.SemaphoreType.DMA((9,)),
        pltpu.SemaphoreType.DMA((2 * NFC,)),
        pltpu.SemaphoreType.DMA((N,)),
        pltpu.SemaphoreType.DMA((N,)),
    ]
    return pl.pallas_call(
        kernel,
        out_shape=jax.ShapeDtypeStruct((B, T, D), x.dtype),
        in_specs=[any_spec] * 12,
        out_specs=any_spec,
        scratch_shapes=scratch,
        compiler_params=pltpu.CompilerParams(vmem_limit_bytes=CFG['vmem_mb'] * 1024 * 1024, flags=CFG['flags']),
    )(x, w_ff1_a, w_ff1_b, w_q, w_k, w_v, w_o, w_pw1, dw, w_pw2, w_ff2_a, w_ff2_b)
```

```python
import math

import jax
import jax.numpy as jnp
from jax import lax
import jax.experimental.pallas as pl
import jax.experimental.pallas.tpu as pltpu

F32 = jnp.float32
BF16 = jnp.bfloat16
EPS = 1e-5
LANES = 128
TM = 400
FC = 512
KC = 512
RB = 40
HALO = 8
CONV_CHUNKS = 5
STAT_GROUPS = 10


def _layernorm(x, post=1.0):
    mu = jnp.mean(x, axis=-1, keepdims=True)
    xc = x - mu
    var = jnp.mean(xc * xc, axis=-1, keepdims=True)
    inv = lax.rsqrt(var + EPS)
    if post != 1.0:
        inv = inv * post
    return xc * inv


def _silu_half(u):
    return u + u * jnp.tanh(u)


def _dot(a, b):
    return jnp.dot(a, b, preferred_element_type=F32)


def _dot_nt(a, b):
    return lax.dot_general(a, b, (((1,), (1,)), ((), ())), preferred_element_type=F32)


def _total(vals):
    t = None
    for v in vals:
        t = v if t is None else t + v
    return t


def _pack_cols(v):
    return [pltpu.bitcast(v[:, c * LANES:(c + 1) * LANES], jnp.uint32) for c in range(v.shape[1] // LANES)]


def _unpack_cols(chunks):
    return jnp.concatenate([pltpu.bitcast(c, BF16) for c in chunks], axis=1)


def _tie32(x, on):
    if on is None:
        return x
    top = x[0:8, 0:LANES] + 0.0 * on
    row0 = jnp.concatenate([top, x[0:8, LANES:]], axis=1) if x.shape[1] > LANES else top
    return jnp.concatenate([row0, x[8:, :]], axis=0)


def _tie_bf16(x32, xb, on):
    if on is None:
        return xb
    z = 0.0 * on
    top = jnp.concatenate([x32[0:8, :] + z, x32[8:16, :] + z], axis=0).astype(BF16)
    row0 = jnp.concatenate([top, xb[0:16, LANES:]], axis=1)
    return jnp.concatenate([row0, xb[16:, :]], axis=0)


def _result_vreg(res, pos):
    nt, r = divmod(pos, res.shape[0] // 8)
    return res[r * 8:(r + 1) * 8, nt * LANES:(nt + 1) * LANES]


def _pace_rows(x, res):
    if res is None:
        return x
    nt = res.shape[1] // LANES
    pace = jnp.concatenate([_result_vreg(res, r * nt) for r in range(res.shape[0] // 8)], axis=0)
    return jnp.concatenate([x[:, 0:LANES] + 0.0 * pace, x[:, LANES:]], axis=1)


@jax.jit
def pallas_standalone__conformer_family_conformer__speech_kernel(
    x, w_ff1_a, w_ff1_b, w_q, w_k, w_v, w_o, w_pw1, dw, w_pw2, w_ff2_a, w_ff2_b,
):
    B, T, D = x.shape
    Fd = w_ff1_a.shape[1]
    K = dw.shape[0]
    NT = T // TM
    N = B * NT
    NFC = Fd // FC
    TP = pl.cdiv(T, KC) * KC
    NKC = TP // KC
    PAD = K // 2
    GROWS = T + 2 * HALO
    NCC = D // LANES
    NBLK = TM // RB
    NCONV = NCC * NBLK
    assert T % TM == 0 and N % 2 == 0 and N >= 6 and K <= 2 * HALO - 1 and NFC == 4
    assert CONV_CHUNKS * KC <= T and NKC > CONV_CHUNKS
    qscale = (D ** -0.5) * math.log2(math.e)

    def rows(i):
        return pl.ds(pl.multiple_of(i * TM, 16), TM)

    def bt(i):
        b = i // NT
        return b, pl.multiple_of((i - b * NT) * TM, 16)

    def kernel(x_hbm, w1a_h, w1b_h, wq_h, wk_h, wv_h, wo_h, wp1_h, dw_h, wp2_h, w2a_h, w2b_h,
               o_hbm,
               xv, w1a, w1b, wq, wk, wv, wo, wp1, dwv, wp2, w2a, w2b,
               m_ref, wvo_ref, res_ref, h_ref, s2, g_ref, dc_ref, st_ref,
               hc_a, hc_b, x3_a, x3_b, mx2, hbuf,
               wsem, csem, xsem, osem):
        wcp = [pltpu.make_async_copy(s, d, wsem.at[i]) for i, (s, d) in enumerate([
            (wq_h, wq), (wk_h, wk), (wv_h, wv), (wo_h, wo), (wp1_h, wp1), (dw_h, dwv), (wp2_h, wp2),
            (w2a_h, w2a), (w2b_h, w2b)])]
        WQ, WK, WV, WO, WP1, DW, WP2, W2A, W2B = range(9)
        acp = [pltpu.make_async_copy(w1a_h.at[:, pl.ds(c * FC, FC)], w1a.at[:, pl.ds(c * FC, FC)], csem.at[c])
               for c in range(NFC)]
        bcp = [pltpu.make_async_copy(w1b_h.at[pl.ds(c * FC, FC)], w1b.at[pl.ds(c * FC, FC)], csem.at[NFC + c])
               for c in range(NFC)]

        def xrows(i, n, k):
            r = pl.ds(pl.multiple_of(i * TM, 16), n * TM)
            return pltpu.make_async_copy(x_hbm.at[r], xv.at[r], xsem.at[k])

        def xpair(j):
            return xrows(2 * j - 1, 2, j + 1)

        xfirst = [xrows(i, 1, i) for i in range(3)]
        xlast = xrows(N - 1, 1, N // 2 + 1)

        def ocopy(i, n, k):
            r = pl.ds(pl.multiple_of(i * TM, 16), n * TM)
            return pltpu.make_async_copy(xv.at[r], o_hbm.at[r], osem.at[k])

        xfirst[0].start()
        acp[0].start()
        bcp[0].start()

        zrow = jnp.zeros((HALO, LANES), F32)
        for b in range(B):
            for cc in range(NCC):
                h_ref[b, cc, T // 2:TP // 2, :] = jnp.zeros(((TP - T) // 2, LANES), jnp.uint32)
                g_ref[b, cc, 0:HALO, :] = zrow
                g_ref[b, cc, HALO + T:GROWS, :] = zrow
        for cc in range(NCC):
            g_ref[0, cc, HALO:2 * HALO + TM, :] = jnp.zeros((TM + HALO, LANES), F32)

        def h_load(b, start, size):
            half = start // 2 if isinstance(start, int) else pl.multiple_of(start // 2, 8)
            return _unpack_cols([h_ref[b, cc, pl.ds(half, size // 2), :] for cc in range(NCC)])

        def w_load(ref):
            return _unpack_cols([ref[cc] for cc in range(NCC)])

        def w_store(ref, v):
            for cc, ch in enumerate(_pack_cols(v)):
                ref[cc] = ch

        def ffn(h_half, wa_ref, wb_ref, hooks, before_up=None, before_down=None):
            y = None
            for c in range(NFC):
                if before_up is not None:
                    before_up(c)
                u = _dot(h_half, wa_ref[:, c * FC:(c + 1) * FC])
                if c in hooks:
                    hooks[c](u)
                a = _silu_half(u).astype(BF16)
                if before_down is not None:
                    before_down(c)
                yc = _dot(a, wb_ref[c * FC:(c + 1) * FC, :])
                y = yc if y is None else y + yc
            return y

        def ln_in(i, pace=None):
            return _layernorm(_pace_rows(xv[rows(i), :].astype(F32), pace), 0.5).astype(BF16)

        def h_store(i, pace=None):
            b, t0 = bt(i)
            hv = _layernorm(_pace_rows(res_ref[rows(i), :], pace)).astype(BF16)
            for cc, ch in enumerate(_pack_cols(hv)):
                h_ref[b, cc, pl.ds(pl.multiple_of(t0 // 2, 8), TM // 2), :] = ch

        def a_tile(i, cur, first=False):
            def next_h(u):
                hbuf[1 - cur] = ln_in(jnp.minimum(i + 1, N - 1), u)

            if first:
                def before_up(c):
                    acp[c].wait()
                    if c >= 2:
                        bcp[c].wait()
                    if c == 0:
                        for cp in (acp[2], bcp[2], acp[3], bcp[3], xfirst[2]):
                            cp.start()
                    if c == 1:
                        for k in (WQ, WK, WV, WO):
                            wcp[k].start()
                    if c == 2:
                        xfirst[1].wait()
                        for j in range(2, N // 2):
                            xpair(j).start()
                        xlast.start()
                        for k in (WP1, DW, WP2, W2A, W2B):
                            wcp[k].start()

                y = ffn(hbuf[cur], w1a, w1b, {2: next_h}, before_up,
                        lambda c: bcp[c].wait() if c < 2 else None)
            else:
                y = ffn(hbuf[cur], w1a, w1b, {1: next_h, 2: lambda u: h_store(i - 1, u)})
            res_ref[rows(i), :] = xv[rows(i), :].astype(F32) + 0.5 * y

        xfirst[0].wait()
        acp[1].start()
        bcp[1].start()
        xfirst[1].start()
        hbuf[0] = ln_in(0)
        a_tile(0, 0, first=True)
        xfirst[2].wait()
        a_tile(1, 1)
        xpair(2).wait()

        def phase_a(j, carry):
            a_tile(2 * j, 0)
            a_tile(2 * j + 1, 1)

            @pl.when(j + 2 < N // 2)
            def _():
                xpair(j + 2).wait()

            @pl.when(j + 2 == N // 2)
            def _():
                xlast.wait()
            return carry

        lax.fori_loop(1, N // 2, phase_a, 0)

        for k in (WQ, WK, WV, WO):
            wcp[k].wait()
        w_store(m_ref, (_dot_nt(wq[...], wk[...]) * qscale).astype(BF16))
        w_store(wvo_ref, _dot(wv[...], wo[...]).astype(BF16))
        h_store(N - 1)
        wcp[WP1].wait()
        wcp[DW].wait()

        def score_chunk(i, c, q, s_ref, mx):
            s = _dot_nt(q, h_load(i // NT, c * KC, KC))
            if (c + 1) * KC > T:
                col = lax.broadcasted_iota(jnp.int32, (TM, KC), 1)
                s = jnp.where(col < T - c * KC, s, -jnp.inf)
            s_ref[:, c * KC:(c + 1) * KC] = s
            for j in range(KC // LANES):
                sj = s[:, j * LANES:(j + 1) * LANES]
                mx = sj if mx is None else jnp.maximum(mx, sj)
            return mx, s

        def pv_chunk(i, c, s_ref, mrow, o, ls, pace):
            if pace is not None:
                mrow = mrow + 0.0 * pace
            p = jnp.exp2(s_ref[:, c * KC:(c + 1) * KC] - jnp.concatenate([mrow] * (KC // LANES), axis=1))
            for j in range(KC // LANES):
                pj = p[:, j * LANES:(j + 1) * LANES]
                ls = pj if ls is None else ls + pj
            oc = _dot(p.astype(BF16), h_load(i // NT, c * KC, KC))
            return (oc if o is None else o + oc), ls, oc

        def conv_block(i, k, pace=None):
            b, t0 = bt(i)
            cc, rb = divmod(k, NBLK)
            off = rb * RB
            dwf = dwv[:, cc * LANES:(cc + 1) * LANES].astype(F32)
            w = [jnp.broadcast_to(dwf[kk:kk + 1, :], (8, LANES)) for kk in range(K)]
            acc = None
            if pace is not None:
                wt = [jnp.concatenate([wk] * (RB // 8 + 1), axis=0) for wk in w]
                zt = jnp.concatenate([0.0 * pace] * (RB // 8 + 1), axis=0)
                ga = [g_ref[b, cc, pl.ds(pl.multiple_of(t0 + (off + 8 * a), 8), RB + 8), :] + zt
                      for a in range(2)]
                for sft in range(8):
                    zs = None
                    for a in range(2):
                        kk = 8 * a + sft - (HALO - PAD)
                        if 0 <= kk < K:
                            term = ga[a] * wt[kk]
                            zs = term if zs is None else zs + term
                    part = zs[sft:sft + RB, :]
                    acc = part if acc is None else acc + part
            else:
                wt = [jnp.concatenate([wk] * (RB // 8), axis=0) for wk in w]
                for kk in range(K):
                    term = g_ref[b, cc, pl.ds(t0 + (off + HALO - PAD + kk), RB), :] * wt[kk]
                    acc = term if acc is None else acc + term
            dc_ref[pl.ds(pl.multiple_of(i * TM + off, 8), RB), cc * LANES:(cc + 1) * LANES] = acc
            return _total([acc[j * 8:(j + 1) * 8, :] for j in range(RB // 8)])

        def conv_jobs(jobs, res):
            nres = (res.shape[1] // LANES) * (TM // 8)
            return [conv_block(ti, k, _result_vreg(res, n * nres // len(jobs)))
                    for n, (ti, k) in enumerate(jobs)]

        def conv_stats(i, sums, pace=None):
            means, m2s = [], []
            grows = TM // STAT_GROUPS
            for cc in range(NCC):
                sc = _total(sums[cc * NBLK:(cc + 1) * NBLK])
                mean_c = jnp.sum(sc, axis=0, keepdims=True) * (1.0 / TM)
                means.append(mean_c)
                mean_b = jnp.broadcast_to(mean_c, (8, LANES))
                acc = None
                for gi in range(STAT_GROUPS):
                    mb = mean_b
                    if pace is not None:
                        nres = (pace.shape[1] // LANES) * (TM // 8)
                        mb = mb + 0.0 * _result_vreg(pace, (cc * STAT_GROUPS + gi) * nres // (NCC * STAT_GROUPS))
                    blk = dc_ref[pl.ds(pl.multiple_of(i * TM + gi * grows, 8), grows), cc * LANES:(cc + 1) * LANES]
                    for j in range(grows // 8):
                        d = blk[j * 8:(j + 1) * 8, :] - mb
                        acc = d * d if acc is None else acc + d * d
                m2s.append(jnp.sum(acc, axis=0, keepdims=True))
            st_ref[i, 0:1, :] = jnp.concatenate(means, axis=1)
            st_ref[i, 1:2, :] = jnp.concatenate(m2s, axis=1)
            return jnp.broadcast_to(m2s[-1], (8, LANES))

        def step(inext, s_next, icur, s_cur, mx_cur, iconv, xconv=None):
            box = dict(mx=None, sidx=0)
            sums = []
            q32 = q = qfull = None
            if inext is not None:
                b, t0 = bt(inext)
                qfull = _dot(h_load(b, t0, TM), w_load(m_ref))
                q32 = qfull[0:16, 0:LANES]
                q = qfull.astype(BF16)

            def do_scores(n, tie=None):
                for _ in range(n):
                    c = box['sidx']
                    if inext is None or c >= NKC:
                        return
                    if c == NKC - 1 and iconv is not None:
                        tie = _total(sums) if tie is None else tie + _total(sums)
                    box['mx'], s = score_chunk(inext, c, _tie_bf16(q32, q, tie), s_next, box['mx'])
                    if iconv is not None and c < CONV_CHUNKS:
                        ks = range(c * NCONV // CONV_CHUNKS, (c + 1) * NCONV // CONV_CHUNKS)
                        sums.extend(conv_jobs([(iconv, k) for k in ks], s))
                    box['sidx'] = c + 1

            if icur is None:
                do_scores(NKC)
                return box['mx']

            mrow = jnp.broadcast_to(jnp.max(mx_cur, axis=-1, keepdims=True), (TM, LANES))
            o = ls = None
            prev = qfull
            xsums = {}
            for c in range(NKC):
                pace = None if prev is None else prev[:, LANES:2 * LANES]
                o, ls, prev = pv_chunk(icur, c, s_cur, mrow, o, ls, pace)
                if inext is None and c < NKC - 1:
                    own = [(iconv, k) for k in range(c * NCONV // (NKC - 1), (c + 1) * NCONV // (NKC - 1))]
                    xj = [(xconv, k) for k in range(NCONV) if (k + 1) % NBLK != 0]
                    jobs = own + xj[c * len(xj) // (NKC - 1):(c + 1) * len(xj) // (NKC - 1)]
                    order = sorted(range(len(jobs)), key=lambda n: n / len(own) if n < len(own)
                                   else (n - len(own) + 0.5) / (len(jobs) - len(own)))
                    vals = dict(zip(order, conv_jobs([jobs[n] for n in order], prev)))
                    sums.extend(vals[n] for n in range(len(own)))
                    xsums.update({jobs[n][1]: vals[n] for n in range(len(own), len(jobs))})
            pv_done = prev[0:8, 0:LANES]
            do_scores(NKC - 3)
            do_scores(1, pv_done)

            lrow = jnp.sum(ls, axis=-1, keepdims=True)
            o = _tie32(o * (1.0 / lrow), _total(sums) if inext is None else None)
            attn = _dot(o.astype(BF16), w_load(wvo_ref))
            x2 = res_ref[rows(icur), :] + attn
            res_ref[rows(icur), :] = x2
            do_scores(1, attn[0:8, 0:LANES])

            tie = conv_stats(iconv, sums, prev) if inext is None else None
            b, t0 = bt(icur)
            pw = _dot(_tie32(_layernorm(x2), tie).astype(BF16), wp1[...])
            g = pw[:, :D] * (0.5 + 0.5 * jnp.tanh(0.5 * pw[:, D:]))
            for cc in range(NCC):
                g_ref[b, cc, pl.ds(pl.multiple_of(t0 + HALO, 8), TM), :] = g[:, cc * LANES:(cc + 1) * LANES]
            if inext is None:
                return xsums
            do_scores(1, pw[0:8, 0:LANES])
            return _tie32(box['mx'], conv_stats(iconv, sums, pw))

        mx2[0] = step(0, s2.at[0], None, None, None, None)

        def phase_b(i, carry):
            cur = i % 2
            nxt = 1 - cur
            mx2[nxt] = step(i + 1, s2.at[nxt], i, s2.at[cur], mx2[cur], jnp.maximum(i - 2, 0))
            return carry

        lax.fori_loop(0, N - 1, phase_b, 0)
        xs = step(None, None, N - 1, s2.at[(N - 1) % 2], mx2[(N - 1) % 2], N - 3, xconv=N - 2)
        for k in range(NCONV):
            if k not in xs:
                xs[k] = conv_block(N - 2, k)
        conv_stats(N - 1, [conv_block(N - 1, k) for k in range(NCONV)])
        conv_stats(N - 2, [xs[k] for k in range(NCONV)])

        means = st_ref[:, 0, :]
        mean = jnp.mean(means, axis=0, keepdims=True)
        dm = means - mean
        m2 = jnp.sum(st_ref[:, 1, :] + dm * dm * float(TM), axis=0, keepdims=True)
        bn_half = 0.5 * lax.rsqrt(m2 * (1.0 / (B * T)) + EPS)

        wcp[WP2].wait()
        wcp[W2A].wait()
        wcp[W2B].wait()

        def c_proj(i, pace=None):
            u = (_pace_rows(dc_ref[rows(i), :], pace) - mean) * bn_half
            return res_ref[rows(i), :] + _dot(_silu_half(u).astype(BF16), wp2[...])

        def c_norm(x3, slot, pace=None):
            slot[0][...] = x3
            slot[1][...] = _layernorm(_pace_rows(x3, pace), 0.5).astype(BF16)

        def out_store(i, pace=None):
            xv[rows(i), :] = _layernorm(_pace_rows(res_ref[rows(i), :], pace)).astype(BF16)

        def c_tile(i, cur, nxt, do_next=True, do_out=True):
            box = {}
            hooks = {}
            if do_next:
                hooks[0] = lambda u: box.update(x3=c_proj(i + 1, u))
                hooks[1] = lambda u: c_norm(box['x3'], nxt, u)
            if do_out:
                hooks[2] = lambda u: out_store(i - 1, u)
            y = ffn(cur[1][...], w2a, w2b, hooks)
            res_ref[rows(i), :] = cur[0][...] + 0.5 * y

        slot_a, slot_b = (x3_a, hc_a), (x3_b, hc_b)

        def c_pair(i, first=False, last=False):
            c_tile(i, slot_a, slot_b, True, not first)
            c_tile(i + 1, slot_b, slot_a, not last, True)
            (ocopy(0, 1, 0) if first else ocopy(i - 1, 2, i // 2)).start()

        def phase_c(j, carry):
            c_pair(2 * j)
            return carry

        c_norm(c_proj(0), slot_a)
        c_pair(0, first=True)
        lax.fori_loop(1, N // 2 - 1, phase_c, 0)
        c_pair(N - 2, last=True)
        out_store(N - 1)
        ocopy(N - 1, 1, N // 2).start()
        ocopy(0, 1, 0).wait()
        for j in range(1, N // 2):
            ocopy(2 * j - 1, 2, j).wait()
        ocopy(N - 1, 1, N // 2).wait()

    any_spec = pl.BlockSpec(memory_space=pl.ANY)
    scratch = [
        pltpu.VMEM((B * T, D), BF16),
        pltpu.VMEM((D, Fd), BF16), pltpu.VMEM((Fd, D), BF16),
        pltpu.VMEM((D, D), BF16), pltpu.VMEM((D, D), BF16), pltpu.VMEM((D, D), BF16), pltpu.VMEM((D, D), BF16),
        pltpu.VMEM((D, 2 * D), BF16), pltpu.VMEM((K, D), BF16), pltpu.VMEM((D, D), BF16),
        pltpu.VMEM((D, Fd), BF16), pltpu.VMEM((Fd, D), BF16),
        pltpu.VMEM((NCC, D // 2, LANES), jnp.uint32),
        pltpu.VMEM((NCC, D // 2, LANES), jnp.uint32),
        pltpu.VMEM((B * T, D), F32),
        pltpu.VMEM((B, NCC, TP // 2, LANES), jnp.uint32),
        pltpu.VMEM((2, TM, TP), F32),
        pltpu.VMEM((B, NCC, GROWS, LANES), F32),
        pltpu.VMEM((B * T, D), F32),
        pltpu.VMEM((N, 8, D), F32),
        pltpu.VMEM((TM, D), BF16), pltpu.VMEM((TM, D), BF16),
        pltpu.VMEM((TM, D), F32), pltpu.VMEM((TM, D), F32),
        pltpu.VMEM((2, TM, LANES), F32),
        pltpu.VMEM((2, TM, D), BF16),
        pltpu.SemaphoreType.DMA((9,)),
        pltpu.SemaphoreType.DMA((2 * NFC,)),
        pltpu.SemaphoreType.DMA((N,)),
        pltpu.SemaphoreType.DMA((N,)),
    ]
    out = pl.pallas_call(
        kernel,
        out_shape=jax.ShapeDtypeStruct((B * T, D), x.dtype),
        in_specs=[any_spec] * 12,
        out_specs=any_spec,
        scratch_shapes=scratch,
        compiler_params=pltpu.CompilerParams(
            vmem_limit_bytes=120 * 1024 * 1024,
            flags={'XLA_TPU_EVENLY_DISTRIBUTE_CRITICAL_NODES': True}),
    )(x.reshape(B * T, D), w_ff1_a, w_ff1_b, w_q, w_k, w_v, w_o, w_pw1, dw, w_pw2, w_ff2_a, w_ff2_b)
    return out.reshape(B, T, D)
```

```python
import math

import jax
import jax.numpy as jnp
from jax import lax
import jax.experimental.pallas as pl
import jax.experimental.pallas.tpu as pltpu

F32 = jnp.float32
BF16 = jnp.bfloat16
EPS = 1e-5
LANES = 128
TM = 400
FC = 512
KC = 512
RB = 40
HALO = 8
CONV_CHUNKS = 4
STAT_GROUPS = 10


def _layernorm(x, post=1.0):
    mu = jnp.mean(x, axis=-1, keepdims=True)
    xc = x - mu
    var = jnp.mean(xc * xc, axis=-1, keepdims=True)
    inv = lax.rsqrt(var + EPS)
    if post != 1.0:
        inv = inv * post
    return xc * inv


def _silu_half(u):
    return u + u * jnp.tanh(u)


def _dot(a, b):
    return jnp.dot(a, b, preferred_element_type=F32)


def _dot_nt(a, b):
    return lax.dot_general(a, b, (((1,), (1,)), ((), ())), preferred_element_type=F32)


def _total(vals):
    t = None
    for v in vals:
        t = v if t is None else t + v
    return t


def _pack_cols(v):
    return [pltpu.bitcast(v[:, c * LANES:(c + 1) * LANES], jnp.uint32) for c in range(v.shape[1] // LANES)]


def _unpack_cols(chunks):
    return jnp.concatenate([pltpu.bitcast(c, BF16) for c in chunks], axis=1)


def _tie32(x, on):
    if on is None:
        return x
    top = x[0:8, 0:LANES] + 0.0 * on
    row0 = jnp.concatenate([top, x[0:8, LANES:]], axis=1) if x.shape[1] > LANES else top
    return jnp.concatenate([row0, x[8:, :]], axis=0)


def _tie_bf16(x32, xb, on):
    if on is None:
        return xb
    z = 0.0 * on
    top = jnp.concatenate([x32[0:8, :] + z, x32[8:16, :] + z], axis=0).astype(BF16)
    row0 = jnp.concatenate([top, xb[0:16, LANES:]], axis=1)
    return jnp.concatenate([row0, xb[16:, :]], axis=0)


def _result_vreg(res, pos):
    nt, r = divmod(pos, res.shape[0] // 8)
    return res[r * 8:(r + 1) * 8, nt * LANES:(nt + 1) * LANES]


def _pace_rows(x, res):
    if res is None:
        return x
    nt = res.shape[1] // LANES
    pace = jnp.concatenate([_result_vreg(res, r * nt) for r in range(res.shape[0] // 8)], axis=0)
    return jnp.concatenate([x[:, 0:LANES] + 0.0 * pace, x[:, LANES:]], axis=1)


@jax.jit
def pallas_standalone__conformer_family_conformer__speech_kernel(
    x, w_ff1_a, w_ff1_b, w_q, w_k, w_v, w_o, w_pw1, dw, w_pw2, w_ff2_a, w_ff2_b,
):
    B, T, D = x.shape
    Fd = w_ff1_a.shape[1]
    K = dw.shape[0]
    NT = T // TM
    N = B * NT
    NFC = Fd // FC
    TP = pl.cdiv(T, KC) * KC
    NKC = TP // KC
    PAD = K // 2
    GROWS = T + 2 * HALO
    NCC = D // LANES
    NBLK = TM // RB
    NCONV = NCC * NBLK
    assert T % TM == 0 and N % 2 == 0 and N >= 6 and K <= 2 * HALO - 1 and NFC == 4
    assert CONV_CHUNKS * KC <= T and NKC > CONV_CHUNKS
    qscale = (D ** -0.5) * math.log2(math.e)

    def rows(i):
        return pl.ds(pl.multiple_of(i * TM, 16), TM)

    def bt(i):
        b = i // NT
        return b, pl.multiple_of((i - b * NT) * TM, 16)

    def kernel(x_hbm, w1a_h, w1b_h, wq_h, wk_h, wv_h, wo_h, wp1_h, dw_h, wp2_h, w2a_h, w2b_h,
               o_hbm,
               xv, w1a, w1b, wq, wk, wv, wo, wp1, dwv, wp2, w2a, w2b,
               m_ref, wvo_ref, res_ref, h_ref, s2, g_ref, dc_ref, st_ref,
               hc_a, hc_b, x3_a, x3_b, mx2, hbuf,
               wsem, csem, xsem, osem):
        wcp = [pltpu.make_async_copy(s, d, wsem.at[i]) for i, (s, d) in enumerate([
            (wq_h, wq), (wk_h, wk), (wv_h, wv), (wo_h, wo), (wp1_h, wp1), (dw_h, dwv), (wp2_h, wp2),
            (w2a_h, w2a), (w2b_h, w2b)])]
        WQ, WK, WV, WO, WP1, DW, WP2, W2A, W2B = range(9)
        acp = [pltpu.make_async_copy(w1a_h.at[:, pl.ds(c * FC, FC)], w1a.at[:, pl.ds(c * FC, FC)], csem.at[c])
               for c in range(NFC)]
        bcp = [pltpu.make_async_copy(w1b_h.at[pl.ds(c * FC, FC)], w1b.at[pl.ds(c * FC, FC)], csem.at[NFC + c])
               for c in range(NFC)]

        def xrows(i, n, k):
            r = pl.ds(pl.multiple_of(i * TM, 16), n * TM)
            return pltpu.make_async_copy(x_hbm.at[r], xv.at[r], xsem.at[k])

        def xpair(j):
            return xrows(2 * j - 1, 2, j + 1)

        xfirst = [xrows(i, 1, i) for i in range(3)]
        xlast = xrows(N - 1, 1, N // 2 + 1)

        def ocopy(i, n, k):
            r = pl.ds(pl.multiple_of(i * TM, 16), n * TM)
            return pltpu.make_async_copy(xv.at[r], o_hbm.at[r], osem.at[k])

        xfirst[0].start()
        acp[0].start()
        bcp[0].start()

        zrow = jnp.zeros((HALO, LANES), F32)
        for b in range(B):
            for cc in range(NCC):
                h_ref[b, cc, T // 2:TP // 2, :] = jnp.zeros(((TP - T) // 2, LANES), jnp.uint32)
                g_ref[b, cc, 0:HALO, :] = zrow
                g_ref[b, cc, HALO + T:GROWS, :] = zrow
        for cc in range(NCC):
            g_ref[0, cc, HALO:2 * HALO + TM, :] = jnp.zeros((TM + HALO, LANES), F32)

        def h_load(b, start, size):
            half = start // 2 if isinstance(start, int) else pl.multiple_of(start // 2, 8)
            return _unpack_cols([h_ref[b, cc, pl.ds(half, size // 2), :] for cc in range(NCC)])

        def w_load(ref):
            return _unpack_cols([ref[cc] for cc in range(NCC)])

        def w_store(ref, v):
            for cc, ch in enumerate(_pack_cols(v)):
                ref[cc] = ch

        def ffn(h_half, wa_ref, wb_ref, hooks, before_up=None, before_down=None):
            y = None
            for c in range(NFC):
                if before_up is not None:
                    before_up(c)
                u = _dot(h_half, wa_ref[:, c * FC:(c + 1) * FC])
                if c in hooks:
                    hooks[c](u)
                a = _silu_half(u).astype(BF16)
                if before_down is not None:
                    before_down(c)
                yc = _dot(a, wb_ref[c * FC:(c + 1) * FC, :])
                y = yc if y is None else y + yc
            return y

        def ln_in(i, pace=None):
            return _layernorm(_pace_rows(xv[rows(i), :].astype(F32), pace), 0.5).astype(BF16)

        def h_store(i, pace=None):
            b, t0 = bt(i)
            hv = _layernorm(_pace_rows(res_ref[rows(i), :], pace)).astype(BF16)
            for cc, ch in enumerate(_pack_cols(hv)):
                h_ref[b, cc, pl.ds(pl.multiple_of(t0 // 2, 8), TM // 2), :] = ch

        def a_tile(i, cur, first=False):
            def next_h(u):
                hbuf[1 - cur] = ln_in(jnp.minimum(i + 1, N - 1), u)

            if first:
                def before_up(c):
                    acp[c].wait()
                    if c >= 2:
                        bcp[c].wait()
                    if c == 0:
                        for cp in (acp[2], bcp[2], acp[3], bcp[3], xfirst[2]):
                            cp.start()
                    if c == 1:
                        for k in (WQ, WK, WV, WO):
                            wcp[k].start()
                    if c == 2:
                        xfirst[1].wait()
                        for j in range(2, N // 2):
                            xpair(j).start()
                        xlast.start()
                        for k in (WP1, DW, WP2, W2A, W2B):
                            wcp[k].start()

                y = ffn(hbuf[cur], w1a, w1b, {2: next_h}, before_up,
                        lambda c: bcp[c].wait() if c < 2 else None)
            else:
                y = ffn(hbuf[cur], w1a, w1b, {1: next_h, 2: lambda u: h_store(i - 1, u)})
            res_ref[rows(i), :] = xv[rows(i), :].astype(F32) + 0.5 * y

        xfirst[0].wait()
        acp[1].start()
        bcp[1].start()
        xfirst[1].start()
        hbuf[0] = ln_in(0)
        a_tile(0, 0, first=True)
        xfirst[2].wait()
        a_tile(1, 1)
        xpair(2).wait()

        def phase_a(j, carry):
            a_tile(2 * j, 0)
            a_tile(2 * j + 1, 1)

            @pl.when(j + 2 < N // 2)
            def _():
                xpair(j + 2).wait()

            @pl.when(j + 2 == N // 2)
            def _():
                xlast.wait()
            return carry

        lax.fori_loop(1, N // 2, phase_a, 0)

        for k in (WQ, WK, WV, WO):
            wcp[k].wait()
        w_store(m_ref, (_dot_nt(wq[...], wk[...]) * qscale).astype(BF16))
        w_store(wvo_ref, _dot(wv[...], wo[...]).astype(BF16))
        h_store(N - 1)
        wcp[WP1].wait()
        wcp[DW].wait()

        def score_chunk(i, c, q, s_ref, mx):
            s = _dot_nt(q, h_load(i // NT, c * KC, KC))
            if (c + 1) * KC > T:
                col = lax.broadcasted_iota(jnp.int32, (TM, KC), 1)
                s = jnp.where(col < T - c * KC, s, -jnp.inf)
            s_ref[:, c * KC:(c + 1) * KC] = s
            for j in range(KC // LANES):
                sj = s[:, j * LANES:(j + 1) * LANES]
                mx = sj if mx is None else jnp.maximum(mx, sj)
            return mx, s

        def pv_chunk(i, c, s_ref, mrow, o, ls, pace):
            if pace is not None:
                mrow = mrow + 0.0 * pace
            p = jnp.exp2(s_ref[:, c * KC:(c + 1) * KC] - jnp.concatenate([mrow] * (KC // LANES), axis=1))
            for j in range(KC // LANES):
                pj = p[:, j * LANES:(j + 1) * LANES]
                ls = pj if ls is None else ls + pj
            oc = _dot(p.astype(BF16), h_load(i // NT, c * KC, KC))
            return (oc if o is None else o + oc), ls, oc

        def conv_block(i, k, pace=None):
            b, t0 = bt(i)
            cc, rb = divmod(k, NBLK)
            off = rb * RB
            dwf = dwv[:, cc * LANES:(cc + 1) * LANES].astype(F32)
            w = [jnp.broadcast_to(dwf[kk:kk + 1, :], (8, LANES)) for kk in range(K)]
            acc = None
            if pace is not None:
                wt = [jnp.concatenate([wk] * (RB // 8 + 1), axis=0) for wk in w]
                zt = jnp.concatenate([0.0 * pace] * (RB // 8 + 1), axis=0)
                ga = [g_ref[b, cc, pl.ds(pl.multiple_of(t0 + (off + 8 * a), 8), RB + 8), :] + zt
                      for a in range(2)]
                for sft in range(8):
                    zs = None
                    for a in range(2):
                        kk = 8 * a + sft - (HALO - PAD)
                        if 0 <= kk < K:
                            term = ga[a] * wt[kk]
                            zs = term if zs is None else zs + term
                    part = zs[sft:sft + RB, :]
                    acc = part if acc is None else acc + part
            else:
                wt = [jnp.concatenate([wk] * (RB // 8), axis=0) for wk in w]
                for kk in range(K):
                    term = g_ref[b, cc, pl.ds(t0 + (off + HALO - PAD + kk), RB), :] * wt[kk]
                    acc = term if acc is None else acc + term
            dc_ref[pl.ds(pl.multiple_of(i * TM + off, 8), RB), cc * LANES:(cc + 1) * LANES] = acc
            return _total([acc[j * 8:(j + 1) * 8, :] for j in range(RB // 8)])

        def conv_jobs(jobs, res):
            nres = (res.shape[1] // LANES) * (TM // 8)
            return [conv_block(ti, k, _result_vreg(res, n * nres // len(jobs)))
                    for n, (ti, k) in enumerate(jobs)]

        def conv_stats(i, sums, pace=None):
            means, m2s = [], []
            grows = TM // STAT_GROUPS
            for cc in range(NCC):
                sc = _total(sums[cc * NBLK:(cc + 1) * NBLK])
                mean_c = jnp.sum(sc, axis=0, keepdims=True) * (1.0 / TM)
                means.append(mean_c)
                mean_b = jnp.broadcast_to(mean_c, (8, LANES))
                acc = None
                for gi in range(STAT_GROUPS):
                    mb = mean_b
                    if pace is not None:
                        nres = (pace.shape[1] // LANES) * (TM // 8)
                        mb = mb + 0.0 * _result_vreg(pace, (cc * STAT_GROUPS + gi) * nres // (NCC * STAT_GROUPS))
                    blk = dc_ref[pl.ds(pl.multiple_of(i * TM + gi * grows, 8), grows), cc * LANES:(cc + 1) * LANES]
                    for j in range(grows // 8):
                        d = blk[j * 8:(j + 1) * 8, :] - mb
                        acc = d * d if acc is None else acc + d * d
                m2s.append(jnp.sum(acc, axis=0, keepdims=True))
            st_ref[i, 0:1, :] = jnp.concatenate(means, axis=1)
            st_ref[i, 1:2, :] = jnp.concatenate(m2s, axis=1)
            return jnp.broadcast_to(m2s[-1], (8, LANES))

        def step(inext, s_next, icur, s_cur, mx_cur, iconv, xconv=None):
            box = dict(mx=None, sidx=0)
            sums = []
            q32 = q = qfull = None
            if inext is not None:
                b, t0 = bt(inext)
                qfull = _dot(h_load(b, t0, TM), w_load(m_ref))
                q32 = qfull[0:16, 0:LANES]
                q = qfull.astype(BF16)

            def do_scores(n, tie=None):
                for _ in range(n):
                    c = box['sidx']
                    if inext is None or c >= NKC:
                        return
                    if c == NKC - 1 and iconv is not None:
                        tie = _total(sums) if tie is None else tie + _total(sums)
                    box['mx'], s = score_chunk(inext, c, _tie_bf16(q32, q, tie), s_next, box['mx'])
                    if iconv is not None and c < CONV_CHUNKS:
                        ks = range(c * NCONV // CONV_CHUNKS, (c + 1) * NCONV // CONV_CHUNKS)
                        sums.extend(conv_jobs([(iconv, k) for k in ks], s))
                    box['sidx'] = c + 1

            if icur is None:
                do_scores(NKC)
                return box['mx']

            mrow = jnp.broadcast_to(jnp.max(mx_cur, axis=-1, keepdims=True), (TM, LANES))
            o = ls = None
            prev = qfull
            xsums = {}
            for c in range(NKC):
                pace = None if prev is None else prev[:, LANES:2 * LANES]
                o, ls, prev = pv_chunk(icur, c, s_cur, mrow, o, ls, pace)
                if inext is None and c < NKC - 1:
                    own = [(iconv, k) for k in range(c * NCONV // (NKC - 1), (c + 1) * NCONV // (NKC - 1))]
                    xj = [(xconv, k) for k in range(NCONV) if (k + 1) % NBLK != 0]
                    jobs = own + xj[c * len(xj) // (NKC - 1):(c + 1) * len(xj) // (NKC - 1)]
                    order = sorted(range(len(jobs)), key=lambda n: n / len(own) if n < len(own)
                                   else (n - len(own) + 0.5) / (len(jobs) - len(own)))
                    vals = dict(zip(order, conv_jobs([jobs[n] for n in order], prev)))
                    sums.extend(vals[n] for n in range(len(own)))
                    xsums.update({jobs[n][1]: vals[n] for n in range(len(own), len(jobs))})
            pv_done = prev[0:8, 0:LANES]
            do_scores(NKC - 3)
            do_scores(1, pv_done)

            lrow = jnp.sum(ls, axis=-1, keepdims=True)
            o = _tie32(o * (1.0 / lrow), _total(sums) if inext is None else None)
            attn = _dot(o.astype(BF16), w_load(wvo_ref))
            x2 = res_ref[rows(icur), :] + attn
            res_ref[rows(icur), :] = x2
            do_scores(1, attn[0:8, 0:LANES])

            tie = conv_stats(iconv, sums, prev) if inext is None else None
            b, t0 = bt(icur)
            pw = _dot(_tie32(_layernorm(x2), tie).astype(BF16), wp1[...])
            g = pw[:, :D] * (0.5 + 0.5 * jnp.tanh(0.5 * pw[:, D:]))
            for cc in range(NCC):
                g_ref[b, cc, pl.ds(pl.multiple_of(t0 + HALO, 8), TM), :] = g[:, cc * LANES:(cc + 1) * LANES]
            if inext is None:
                return xsums
            do_scores(1, pw[0:8, 0:LANES])
            return _tie32(box['mx'], conv_stats(iconv, sums, pw))

        mx2[0] = step(0, s2.at[0], None, None, None, None)

        def phase_b(i, carry):
            cur = i % 2
            nxt = 1 - cur
            mx2[nxt] = step(i + 1, s2.at[nxt], i, s2.at[cur], mx2[cur], jnp.maximum(i - 2, 0))
            return carry

        lax.fori_loop(0, N - 1, phase_b, 0)
        xs = step(None, None, N - 1, s2.at[(N - 1) % 2], mx2[(N - 1) % 2], N - 3, xconv=N - 2)
        for k in range(NCONV):
            if k not in xs:
                xs[k] = conv_block(N - 2, k)
        conv_stats(N - 1, [conv_block(N - 1, k) for k in range(NCONV)])
        conv_stats(N - 2, [xs[k] for k in range(NCONV)])

        means = st_ref[:, 0, :]
        mean = jnp.mean(means, axis=0, keepdims=True)
        dm = means - mean
        m2 = jnp.sum(st_ref[:, 1, :] + dm * dm * float(TM), axis=0, keepdims=True)
        bn_half = 0.5 * lax.rsqrt(m2 * (1.0 / (B * T)) + EPS)

        wcp[WP2].wait()
        wcp[W2A].wait()
        wcp[W2B].wait()

        def c_proj(i, pace=None):
            u = (_pace_rows(dc_ref[rows(i), :], pace) - mean) * bn_half
            return res_ref[rows(i), :] + _dot(_silu_half(u).astype(BF16), wp2[...])

        def c_norm(x3, slot, pace=None):
            slot[0][...] = x3
            slot[1][...] = _layernorm(_pace_rows(x3, pace), 0.5).astype(BF16)

        def out_store(i, pace=None):
            xv[rows(i), :] = _layernorm(_pace_rows(res_ref[rows(i), :], pace)).astype(BF16)

        def c_tile(i, cur, nxt, do_next=True, do_out=True):
            box = {}
            hooks = {}
            if do_next:
                hooks[0] = lambda u: box.update(x3=c_proj(i + 1, u))
                hooks[1] = lambda u: c_norm(box['x3'], nxt, u)
            if do_out:
                hooks[2] = lambda u: out_store(i - 1, u)
            y = ffn(cur[1][...], w2a, w2b, hooks)
            res_ref[rows(i), :] = cur[0][...] + 0.5 * y

        slot_a, slot_b = (x3_a, hc_a), (x3_b, hc_b)

        def c_pair(i, first=False, last=False):
            c_tile(i, slot_a, slot_b, True, not first)
            c_tile(i + 1, slot_b, slot_a, not last, True)
            (ocopy(0, 1, 0) if first else ocopy(i - 1, 2, i // 2)).start()

        def phase_c(j, carry):
            c_pair(2 * j)
            return carry

        c_norm(c_proj(0), slot_a)
        c_pair(0, first=True)
        lax.fori_loop(1, N // 2 - 1, phase_c, 0)
        c_pair(N - 2, last=True)
        out_store(N - 1)
        ocopy(N - 1, 1, N // 2).start()
        ocopy(0, 1, 0).wait()
        for j in range(1, N // 2):
            ocopy(2 * j - 1, 2, j).wait()
        ocopy(N - 1, 1, N // 2).wait()

    any_spec = pl.BlockSpec(memory_space=pl.ANY)
    scratch = [
        pltpu.VMEM((B * T, D), BF16),
        pltpu.VMEM((D, Fd), BF16), pltpu.VMEM((Fd, D), BF16),
        pltpu.VMEM((D, D), BF16), pltpu.VMEM((D, D), BF16), pltpu.VMEM((D, D), BF16), pltpu.VMEM((D, D), BF16),
        pltpu.VMEM((D, 2 * D), BF16), pltpu.VMEM((K, D), BF16), pltpu.VMEM((D, D), BF16),
        pltpu.VMEM((D, Fd), BF16), pltpu.VMEM((Fd, D), BF16),
        pltpu.VMEM((NCC, D // 2, LANES), jnp.uint32),
        pltpu.VMEM((NCC, D // 2, LANES), jnp.uint32),
        pltpu.VMEM((B * T, D), F32),
        pltpu.VMEM((B, NCC, TP // 2, LANES), jnp.uint32),
        pltpu.VMEM((2, TM, TP), F32),
        pltpu.VMEM((B, NCC, GROWS, LANES), F32),
        pltpu.VMEM((B * T, D), F32),
        pltpu.VMEM((N, 8, D), F32),
        pltpu.VMEM((TM, D), BF16), pltpu.VMEM((TM, D), BF16),
        pltpu.VMEM((TM, D), F32), pltpu.VMEM((TM, D), F32),
        pltpu.VMEM((2, TM, LANES), F32),
        pltpu.VMEM((2, TM, D), BF16),
        pltpu.SemaphoreType.DMA((9,)),
        pltpu.SemaphoreType.DMA((2 * NFC,)),
        pltpu.SemaphoreType.DMA((N,)),
        pltpu.SemaphoreType.DMA((N,)),
    ]
    out = pl.pallas_call(
        kernel,
        out_shape=jax.ShapeDtypeStruct((B * T, D), x.dtype),
        in_specs=[any_spec] * 12,
        out_specs=any_spec,
        scratch_shapes=scratch,
        compiler_params=pltpu.CompilerParams(vmem_limit_bytes=120 * 1024 * 1024),
    )(x.reshape(B * T, D), w_ff1_a, w_ff1_b, w_q, w_k, w_v, w_o, w_pw1, dw, w_pw2, w_ff2_a, w_ff2_b)
    return out.reshape(B, T, D)
```
